```python
import jax
import jax.numpy as jnp

def _softmax(x, axis=-1):
    return jax.nn.softmax(x, axis=axis)
def _gelu(x):
    return jax.nn.gelu(x, approximate=True)
def _silu(x):
    return jax.nn.silu(x)
def _sigmoid(x):
    return jax.nn.sigmoid(x)
def _layernorm(x, axis=-1, eps=1e-5):
    m = jnp.mean(x, axis=axis, keepdims=True)
    v = jnp.var(x, axis=axis, keepdims=True)
    return (x - m) / jnp.sqrt(v + eps)
def _scatter_add(tgt, idx, src, axis=0):
    return tgt.at[idx].add(src)
def _segment_sum(src, seg, n):
    return jax.ops.segment_sum(src, seg, n)
class _Rng:
    def __init__(self, key):
        self._k = key
    def _next(self):
        self._k, sub = jax.random.split(self._k)
        return sub
    def normal(self, shape):
        return jax.random.normal(self._next(), shape, dtype=jnp.bfloat16)
    def randint(self, lo, hi, shape):
        return jax.random.randint(self._next(), shape, lo, hi, dtype=jnp.int32)
    def uniform(self, shape, lo=0.0, hi=1.0):
        return jax.random.uniform(self._next(), shape, jnp.bfloat16, lo, hi)
    def permutation(self, n):
        return jax.random.permutation(self._next(), n)


kernel_name = 'gated_mix__compressed_kv_cla__gqa_block_cached__decode'

def setup_inputs():
    _rng = _Rng(jax.random.key(int.from_bytes(__import__("os").urandom(4), "little")))
    _w = (lambda a: (lambda t: t.astype(jnp.bfloat16) if jnp.issubdtype(t.dtype, jnp.floating) else t)(jnp.asarray(a)))
    def _A_setup():
        B, H, Sq, Sk, D, M = 1, 32, 1, 4096, 128, 640
        Dc = 4 * D
        return {
            "x": _w((lambda *s: _rng.normal(s) * 0.05)(B, Sq, M)),
            "c_kv": _w((lambda *s: _rng.normal(s) * 0.05)(B, Sk, Dc)),
            "w_q": _w((lambda *s: _rng.normal(s) * 0.05)(M, H, D) * (M ** -0.5)),
            "w_uk": _w((lambda *s: _rng.normal(s) * 0.05)(Dc, H, D) * (Dc ** -0.5)),
            "w_uv": _w((lambda *s: _rng.normal(s) * 0.05)(Dc, H, D) * (Dc ** -0.5)),
            "w_o": _w((lambda *s: _rng.normal(s) * 0.05)(H, D, M) * ((H * D) ** -0.5)),
        }
    _A_in = _A_setup()

    def _B_setup():
        B, Sq, D = 1, 1, 640
        Hq, Hkv, Sk, Dh = 32, 32, 4096, 128
        assert Hq % Hkv == 0, (Hq, Hkv)
        return {
            "x": _w((lambda *s: _rng.normal(s) * 0.05)(B, Sq, D)),
            "k_cache": _w((lambda *s: _rng.normal(s) * 0.05)(B, Hkv, Sk, Dh)),
            "v_cache": _w((lambda *s: _rng.normal(s) * 0.05)(B, Hkv, Sk, Dh)),
            "wq": _w((lambda *s: _rng.normal(s) * 0.05)(D, Hq * Dh) * (D ** -0.5)),
            "wo": _w((lambda *s: _rng.normal(s) * 0.05)(Hq * Dh, D) * ((Hq * Dh) ** -0.5)),
        }
    _B_in = _B_setup()

    return {
        "A_x": _A_in["x"],
        "A_c_kv": _A_in["c_kv"],
        "A_w_q": _A_in["w_q"],
        "A_w_uk": _A_in["w_uk"],
        "A_w_uv": _A_in["w_uv"],
        "A_w_o": _A_in["w_o"],
        "B_x": _B_in["x"],
        "B_k_cache": _B_in["k_cache"],
        "B_v_cache": _B_in["v_cache"],
        "B_wq": _B_in["wq"],
        "B_wo": _B_in["wo"],
        "gate_w": _w((lambda *s: _rng.normal(s) * 0.05)(640)),
    }

def reference(A_x, A_c_kv, A_w_q, A_w_uk, A_w_uv, A_w_o, B_x, B_k_cache, B_v_cache, B_wq, B_wo, gate_w):
    def _A_ref(x, c_kv, w_q, w_uk, w_uv, w_o):
        B, Sq, M = x.shape[0], x.shape[1], x.shape[2]
        Sk = c_kv.shape[1]
        H, D = w_q.shape[1], w_q.shape[2]
        q = jnp.einsum("bqm,mhd->bhqd", x, w_q)
        k = jnp.einsum("bkc,chd->bhkd", c_kv, w_uk)
        v = jnp.einsum("bkc,chd->bhkd", c_kv, w_uv)
        scores = jnp.einsum("bhqd,bhkd->bhqk", q, k) * (D ** -0.5)
        off = Sk - Sq
        qi = jnp.arange(Sq)[:, None]
        kj = jnp.arange(Sk)[None, :]
        cmask = kj <= (qi + off)
        scores = jnp.where(cmask[None, None], scores, -1e9)
        p = _softmax(scores, axis=-1)
        ctx = jnp.einsum("bhqk,bhkd->bhqd", p, v)
        return jnp.einsum("bhqd,hdm->bqm", ctx, w_o)

    def _B_ref(x, k_cache, v_cache, wq, wo):
        B, Sq, D = x.shape
        Hq, Dh = 32, 128
        Hkv = k_cache.shape[1]
        rep = Hq // Hkv
        q = (lambda x, *d: x.transpose(*d))((x @ wq).reshape(B, Sq, Hq, Dh), 0, 2, 1, 3)
        k = jnp.repeat(k_cache, rep, axis=1)
        v = jnp.repeat(v_cache, rep, axis=1)
        scores = jnp.einsum("bhqd,bhkd->bhqk", q, k) * (Dh ** -0.5)
        p = _softmax(scores, axis=-1)
        o = jnp.einsum("bhqk,bhkd->bhqd", p, v)
        return (lambda x, *d: x.transpose(*d))(o, 0, 2, 1, 3).reshape(B, Sq, Hq * Dh) @ wo

    x = A_x
    g = _sigmoid((x * gate_w).sum(-1, keepdims=True))
    a = _A_ref(x, A_c_kv, A_w_q, A_w_uk, A_w_uv, A_w_o)
    b = _B_ref(x, B_k_cache, B_v_cache, B_wq, B_wo)
    return g * a + (1 - g) * b
```

```python
import functools

import jax
import jax.numpy as jnp
import jax.experimental.pallas as pl
import jax.experimental.pallas.tpu as pltpu

F32 = jnp.float32
BF16 = jnp.bfloat16

M = 640
H = 32
D = 128
DC = 512
SK = 4096
ND = 32
SCALE = D ** -0.5

N_P1, N_P2, N_P3, N_P4 = 5, 4, 2, 4


def _kernel(
    x_hbm, ckv_hbm, wqa_hbm, wuk_hbm, wuv_hbm, woa_hbm, k_hbm, v_hbm, wqb_hbm, wob_hbm, gate_hbm,
    o_ref,
    x_v, gate_v, ckv, wqa, wuk, wuv, woa, kb, vb, wqb, wob,
    xcol, qb_acc, q_scr, qa_scr, r_scr, s_scr, cc_scr, ctx_scr, o_scr,
    sem_misc, sem0, sem1, sem_k, sem_v, sem_woa, sem_wob,
):
    def start(src, dst, sem, queue):
        pltpu.make_async_copy(src, dst, sem).start(priority=queue)

    def wait_all(dst, sem):
        pltpu.make_async_copy(dst, dst, sem).wait()

    def issue_loop(fn):
        def body(i, c):
            fn(i)
            return c
        jax.lax.fori_loop(0, ND, body, 0)

    def issue_p1(j):
        def f(i):
            r = pl.multiple_of(j * 128 + (i // 2) * 8, 8)
            c = pl.multiple_of((i % 2) * 2048, 128)
            start(wqb_hbm.at[pl.ds(r, 8), pl.ds(c, 2048)], wqb.at[pl.ds(r, 8), pl.ds(c, 2048)],
                  sem0.at[j], 0)
            m = j * 128 + i * 4
            start(wqa_hbm.at[pl.ds(m, 4)], wqa.at[pl.ds(m, 4)], sem1.at[j], 1)
        issue_loop(f)

    def wait_p1(j):
        wait_all(wqb.at[pl.ds(j * 128, 128), :], sem0.at[j])
        wait_all(wqa.at[pl.ds(j * 128, 128)], sem1.at[j])

    P2 = N_P1

    def issue_p2(j):
        def f(i):
            c = j * 128 + i * 4
            start(wuk_hbm.at[pl.ds(c, 4)], wuk.at[pl.ds(c, 4)], sem0.at[P2 + j], 0)
            r = pl.multiple_of(j * 1024 + i * 32, 32)
            start(ckv_hbm.at[0, pl.ds(r, 32), :], ckv.at[pl.ds(r, 32), :], sem1.at[P2 + j], 1)
        issue_loop(f)

    def wait_p2(j):
        wait_all(wuk.at[pl.ds(j * 128, 128)], sem0.at[P2 + j])
        wait_all(ckv.at[pl.ds(j * 1024, 1024), :], sem1.at[P2 + j])

    P3 = N_P1 + N_P2

    def issue_p3(j):
        def f(i):
            c = j * 128 + i * 4
            start(wuv_hbm.at[pl.ds(c, 4)], wuv.at[pl.ds(c, 4)], sem0.at[P3 + j], 0)
            start(wuv_hbm.at[pl.ds(c + 256, 4)], wuv.at[pl.ds(c + 256, 4)], sem1.at[P3 + j], 1)
        issue_loop(f)

    def wait_p3(j):
        wait_all(wuv.at[pl.ds(j * 128, 128)], sem0.at[P3 + j])
        wait_all(wuv.at[pl.ds(256 + j * 128, 128)], sem1.at[P3 + j])

    def issue_kv(h):
        def f(i):
            r = pl.multiple_of(i * 128, 128)
            start(k_hbm.at[0, h, pl.ds(r, 128), :], kb.at[h, pl.ds(r, 128), :], sem_k.at[h], 0)
            start(v_hbm.at[0, h, pl.ds(r, 128), :], vb.at[h, pl.ds(r, 128), :], sem_v.at[h], 1)
        issue_loop(f)

    def issue_p4(j):
        def f(i):
            h = j * 8 + i // 4
            r = pl.multiple_of((i % 4) * 32, 32)
            start(woa_hbm.at[h, pl.ds(r, 32), :], woa.at[h, pl.ds(r, 32), :], sem_woa.at[h], 0)
            rr = pl.multiple_of(h * 128 + r, 32)
            start(wob_hbm.at[pl.ds(rr, 32), :], wob.at[pl.ds(rr, 32), :], sem_wob.at[h], 1)
        issue_loop(f)

    def stage_p1(j, xb):
        part = jnp.dot(xb[:, j * 128:(j + 1) * 128], wqb[pl.ds(j * 128, 128), :],
                       preferred_element_type=F32)
        if j == 0:
            qb_acc[...] = part
        else:
            qb_acc[...] += part
        unroll = 16

        def body(i, acc):
            for u in range(unroll):
                m = j * 128 + i * unroll + u
                acc = acc + xcol[pl.ds(m, 1), :] * wqa[m].astype(F32)
            return acc
        acc = jax.lax.fori_loop(0, 128 // unroll, body, jnp.zeros((H, D), F32))
        if j == 0:
            qa_scr[...] = acc
        else:
            qa_scr[...] += acc

    def stage_q_finish():
        for h in range(H):
            q_scr[h] = qb_acc[:, h * D:(h + 1) * D]

    def stage_qabs(j):
        q = qa_scr[...]
        lane = jax.lax.broadcasted_iota(jnp.int32, (H, 128), 1)
        unroll = 16

        def body(i, r):
            for u in range(unroll):
                cl = i * unroll + u
                s = jnp.sum(wuk[j * 128 + cl].astype(F32) * q, axis=-1, keepdims=True)
                r = jnp.where(lane == cl, s, r)
            return r
        r_scr[:, j * 128:(j + 1) * 128] = jax.lax.fori_loop(
            0, 128 // unroll, body, jnp.zeros((H, 128), F32))

    KC = 1024

    def stage_a_scores():
        r = r_scr[...].astype(BF16)
        for t in range(SK // KC):
            s = jax.lax.dot_general(r, ckv[pl.ds(t * KC, KC), :], (((1,), (1,)), ((), ())),
                                    preferred_element_type=F32)
            s_scr[:, t * KC:(t + 1) * KC] = s * SCALE

    def stage_a_softmax_pv():
        m = s_scr[:, 0:KC]
        for t in range(1, SK // KC):
            m = jnp.maximum(m, s_scr[:, t * KC:(t + 1) * KC])
        m = jnp.max(m, axis=-1, keepdims=True)
        l = jnp.zeros((H, 1), F32)
        acc = jnp.zeros((H, DC), F32)
        for t in range(SK // KC):
            p = jnp.exp(s_scr[:, t * KC:(t + 1) * KC] - m)
            l = l + jnp.sum(p, axis=-1, keepdims=True)
            acc = acc + jnp.dot(p.astype(BF16), ckv[pl.ds(t * KC, KC), :], preferred_element_type=F32)
        cc = acc / l
        for g in range(DC // 128):
            cc_scr[g] = cc[:, g * 128:(g + 1) * 128]

    def stage_ctx(g):
        cc = cc_scr[g]
        acc = ctx_scr[...]
        for cl in range(128):
            acc = acc + cc[:, cl:cl + 1] * wuv[g * 128 + cl].astype(F32)
        ctx_scr[...] = acc

    def stage_head(h):
        q = q_scr[h].astype(BF16)
        s = jax.lax.dot_general(q, kb[h], (((1,), (1,)), ((), ())), preferred_element_type=F32) * SCALE
        m = jnp.max(s, axis=-1, keepdims=True)
        p = jnp.exp(s - m)
        l = jnp.sum(p, axis=-1, keepdims=True)
        o = jnp.dot(p.astype(BF16), vb[h], preferred_element_type=F32)
        o_scr[h] = o / l

    start(x_hbm, x_v, sem_misc.at[0], 0)
    start(gate_hbm, gate_v, sem_misc.at[1], 1)
    issue_p1(0)
    issue_p1(1)
    wait_all(x_v, sem_misc.at[0])
    wait_all(gate_v, sem_misc.at[1])

    xf = x_v[0].astype(F32)
    xb = jnp.broadcast_to(xf, (8, M)).astype(BF16)
    xcol[...] = jnp.broadcast_to(xf, (128, M)).T
    gsum = jnp.sum(xf * gate_v[...].astype(F32).reshape(1, M), axis=-1, keepdims=True)
    g = jax.nn.sigmoid(gsum)
    ctx_scr[...] = jnp.zeros_like(ctx_scr)

    static_steps = ([("p1", j) for j in range(N_P1)] + [("p2", j) for j in range(N_P2)]
                    + [("p3", j) for j in range(N_P3)])
    n_static = len(static_steps)

    def issue_step(s):
        if s < n_static:
            kind, j = static_steps[s]
            {"p1": issue_p1, "p2": issue_p2, "p3": issue_p3}[kind](j)
        else:
            issue_kv(s - n_static)

    for s, (kind, j) in enumerate(static_steps):
        issue_step(s + 2)
        if kind == "p1":
            wait_p1(j)
            stage_p1(j, xb)
            if j == N_P1 - 1:
                stage_q_finish()
        elif kind == "p2":
            wait_p2(j)
            stage_qabs(j)
        else:
            wait_p3(j)
            if j == 0:
                stage_a_scores()
            else:
                stage_a_softmax_pv()

    def head_body(h, c):
        @pl.when(h < H - 2)
        def _():
            issue_kv(h + 2)

        @pl.when(h >= H - 2)
        def _():
            issue_p4(h - (H - 2))

        wait_all(kb.at[h], sem_k.at[h])
        wait_all(vb.at[h], sem_v.at[h])
        stage_head(h)

        @pl.when(h < DC // 128)
        def _():
            stage_ctx(h)
        return c
    jax.lax.fori_loop(0, H, head_body, 0)

    acc_a = jnp.zeros((8, M), F32)
    acc_b = jnp.zeros((8, M), F32)
    for j in range(N_P4):
        if j + 2 < N_P4:
            issue_p4(j + 2)
        for h in range(8 * j, 8 * j + 8):
            wait_all(woa.at[h], sem_woa.at[h])
            wait_all(wob.at[pl.ds(h * D, D), :], sem_wob.at[h])
            ctx_h = jnp.broadcast_to(ctx_scr[h:h + 1, :], (8, D)).astype(BF16)
            acc_a = acc_a + jnp.dot(ctx_h, woa[h], preferred_element_type=F32)
            acc_b = acc_b + jnp.dot(o_scr[h].astype(BF16), wob[pl.ds(h * D, D), :],
                                    preferred_element_type=F32)

    out = g * acc_a[0:1, :] + (1.0 - g) * acc_b[0:1, :]
    o_ref[0] = out.astype(o_ref.dtype)


@jax.jit
def pallas_gated_mix__compressed_kv_cla__gqa_block_cached__decode_kernel(
    A_x: jax.Array,
    A_c_kv: jax.Array,
    A_w_q: jax.Array,
    A_w_uk: jax.Array,
    A_w_uv: jax.Array,
    A_w_o: jax.Array,
    B_x: jax.Array,
    B_k_cache: jax.Array,
    B_v_cache: jax.Array,
    B_wq: jax.Array,
    B_wo: jax.Array,
    gate_w: jax.Array,
):
    del B_x
    any_spec = pl.BlockSpec(memory_space=pl.ANY)
    dma = pltpu.SemaphoreType.DMA
    n_static = N_P1 + N_P2 + N_P3
    return pl.pallas_call(
        _kernel,
        out_shape=jax.ShapeDtypeStruct((1, 1, M), A_x.dtype),
        in_specs=[any_spec] * 11,
        out_specs=pl.BlockSpec(memory_space=pltpu.VMEM),
        scratch_shapes=[
            pltpu.VMEM((1, 1, M), BF16),
            pltpu.VMEM((M,), BF16),
            pltpu.VMEM((SK, DC), BF16),
            pltpu.VMEM((M, H, D), BF16),
            pltpu.VMEM((DC, H, D), BF16),
            pltpu.VMEM((DC, H, D), BF16),
            pltpu.VMEM((H, D, M), BF16),
            pltpu.VMEM((H, SK, D), BF16),
            pltpu.VMEM((H, SK, D), BF16),
            pltpu.VMEM((M, H * D), BF16),
            pltpu.VMEM((H * D, M), BF16),
            pltpu.VMEM((M, 128), F32),
            pltpu.VMEM((8, H * D), F32),
            pltpu.VMEM((H, 8, D), F32),
            pltpu.VMEM((H, D), F32),
            pltpu.VMEM((H, DC), F32),
            pltpu.VMEM((H, SK), F32),
            pltpu.VMEM((DC // 128, H, 128), F32),
            pltpu.VMEM((H, D), F32),
            pltpu.VMEM((H, 8, D), F32),
            dma((2,)), dma((n_static,)), dma((n_static,)), dma((H,)), dma((H,)), dma((H,)), dma((H,)),
        ],
        compiler_params=pltpu.CompilerParams(vmem_limit_bytes=112 * 1024 * 1024),
    )(A_x, A_c_kv, A_w_q, A_w_uk, A_w_uv, A_w_o, B_k_cache, B_v_cache, B_wq, B_wo, gate_w)
```

```python
import functools

import jax
import jax.numpy as jnp
import jax.experimental.pallas as pl
import jax.experimental.pallas.tpu as pltpu

F32 = jnp.float32
BF16 = jnp.bfloat16

M = 640
H = 32
D = 128
DC = 512
SK = 4096
ND = 32
SCALE = D ** -0.5

N_P1, N_P2, N_P3, N_P4 = 5, 4, 2, 4
RING = 3
LAST_SPLIT = (4, 2, 1, 1)


def _kernel(
    x_hbm, ckv_hbm, wqa_hbm, wuk_hbm, wuv_hbm, woa_hbm, k_hbm, v_hbm, wqb_hbm, wob_hbm, gate_hbm,
    o_ref,
    x_v, gate_v, ckv, wqa, wuk, wuv, woa, kb, vb, wqb, wob,
    xcol, qb_acc, q_scr, qa_scr, r_scr, s_scr, cc_scr, ctx_scr, o_scr,
    sem0, sem1,
):
    def start(src, dst, sem, queue):
        pltpu.make_async_copy(src, dst, sem).start(priority=queue)

    def wait_all(dst, sem):
        pltpu.make_async_copy(dst, dst, sem).wait()

    def issue_loop(fn):
        def body(i, c):
            fn(i)
            return c
        jax.lax.fori_loop(0, ND, body, 0)

    def slot(s):
        return s % RING if isinstance(s, int) else jax.lax.rem(s, RING)

    def issue_p1(j):
        def f(i):
            r = pl.multiple_of(j * 128 + (i // 2) * 8, 8)
            c = pl.multiple_of((i % 2) * 2048, 128)
            start(wqb_hbm.at[pl.ds(r, 8), pl.ds(c, 2048)], wqb.at[pl.ds(r, 8), pl.ds(c, 2048)],
                  sem0.at[slot(j)], 0)
            m = j * 128 + i * 4
            start(wqa_hbm.at[pl.ds(m, 4)], wqa.at[pl.ds(m, 4)], sem1.at[slot(j)], 1)
        issue_loop(f)

    def wait_p1(j):
        wait_all(wqb.at[pl.ds(j * 128, 128), :], sem0.at[slot(j)])
        wait_all(wqa.at[pl.ds(j * 128, 128)], sem1.at[slot(j)])

    P2 = N_P1

    def issue_p2(j):
        def f(i):
            c = j * 128 + i * 4
            start(wuk_hbm.at[pl.ds(c, 4)], wuk.at[pl.ds(c, 4)], sem0.at[slot(P2 + j)], 0)
            r = pl.multiple_of(j * 1024 + i * 32, 32)
            start(ckv_hbm.at[0, pl.ds(r, 32), :], ckv.at[pl.ds(r, 32), :], sem1.at[slot(P2 + j)], 1)
        issue_loop(f)

    def wait_p2(j):
        wait_all(wuk.at[pl.ds(j * 128, 128)], sem0.at[slot(P2 + j)])
        wait_all(ckv.at[pl.ds(j * 1024, 1024), :], sem1.at[slot(P2 + j)])

    P3 = N_P1 + N_P2

    def issue_p3(j):
        def f(i):
            c = j * 128 + i * 4
            start(wuv_hbm.at[pl.ds(c, 4)], wuv.at[pl.ds(c, 4)], sem0.at[slot(P3 + j)], 0)
            start(wuv_hbm.at[pl.ds(c + 256, 4)], wuv.at[pl.ds(c + 256, 4)], sem1.at[slot(P3 + j)], 1)
        issue_loop(f)

    def wait_p3(j):
        wait_all(wuv.at[pl.ds(j * 128, 128)], sem0.at[slot(P3 + j)])
        wait_all(wuv.at[pl.ds(256 + j * 128, 128)], sem1.at[slot(P3 + j)])

    PH = N_P1 + N_P2 + N_P3
    P4 = PH + H

    def issue_kv(h):
        sl = slot(PH + h)

        def f(i):
            r = pl.multiple_of(i * 128, 128)
            start(k_hbm.at[0, h, pl.ds(r, 128), :], kb.at[h, pl.ds(r, 128), :], sem0.at[sl], 0)
            start(v_hbm.at[0, h, pl.ds(r, 128), :], vb.at[h, pl.ds(r, 128), :], sem1.at[sl], 1)
        issue_loop(f)

    def issue_wo(h0, nh, sl):
        def f(i):
            h = h0 + i // 4
            r = pl.multiple_of((i % 4) * 32, 32)
            start(woa_hbm.at[h, pl.ds(r, 32), :], woa.at[h, pl.ds(r, 32), :], sem0.at[sl], 0)
            rr = pl.multiple_of(h * 128 + r, 32)
            start(wob_hbm.at[pl.ds(rr, 32), :], wob.at[pl.ds(rr, 32), :], sem1.at[sl], 1)

        def body(i, c):
            f(i)
            return c
        jax.lax.fori_loop(0, nh * 4, body, 0)

    def wait_wo(h0, nh, sl):
        wait_all(woa.at[pl.ds(h0, nh)], sem0.at[sl])
        wait_all(wob.at[pl.ds(h0 * D, nh * D), :], sem1.at[sl])

    def p4_groups(j):
        if j < N_P4 - 1:
            return [(8 * j, 8, slot(P4 + j))]
        groups, h0 = [], 8 * j
        for n, nh in enumerate(LAST_SPLIT):
            groups.append((h0, nh, slot(P4 + j) if n == 0 else RING + n - 1))
            h0 += nh
        return groups

    def issue_p4(j):
        for h0, nh, sl in p4_groups(j):
            issue_wo(h0, nh, sl)

    def stage_p1(j, xb):
        part = jnp.dot(xb[:, j * 128:(j + 1) * 128], wqb[pl.ds(j * 128, 128), :],
                       preferred_element_type=F32)
        if j == 0:
            qb_acc[...] = part
        else:
            qb_acc[...] += part
        unroll = 16

        def body(i, acc):
            for u in range(unroll):
                m = j * 128 + i * unroll + u
                acc = acc + xcol[pl.ds(m, 1), :] * wqa[m].astype(F32)
            return acc
        acc = jax.lax.fori_loop(0, 128 // unroll, body, jnp.zeros((H, D), F32))
        if j == 0:
            qa_scr[...] = acc
        else:
            qa_scr[...] += acc

    def stage_q_finish():
        for h in range(H):
            q_scr[h] = qb_acc[:, h * D:(h + 1) * D]

    def stage_qabs(j):
        q = qa_scr[...]
        lane = jax.lax.broadcasted_iota(jnp.int32, (H, 128), 1)
        unroll = 16

        def body(i, r):
            for u in range(unroll):
                cl = i * unroll + u
                s = jnp.sum(wuk[j * 128 + cl].astype(F32) * q, axis=-1, keepdims=True)
                r = jnp.where(lane == cl, s, r)
            return r
        r_scr[:, j * 128:(j + 1) * 128] = jax.lax.fori_loop(
            0, 128 // unroll, body, jnp.zeros((H, 128), F32))

    KC = 1024

    def stage_a_scores():
        r = r_scr[...].astype(BF16)
        for t in range(SK // KC):
            s = jax.lax.dot_general(r, ckv[pl.ds(t * KC, KC), :], (((1,), (1,)), ((), ())),
                                    preferred_element_type=F32)
            s_scr[:, t * KC:(t + 1) * KC] = s * SCALE

    def stage_a_softmax_pv():
        m = s_scr[:, 0:KC]
        for t in range(1, SK // KC):
            m = jnp.maximum(m, s_scr[:, t * KC:(t + 1) * KC])
        m = jnp.max(m, axis=-1, keepdims=True)
        l = jnp.zeros((H, 1), F32)
        acc = jnp.zeros((H, DC), F32)
        for t in range(SK // KC):
            p = jnp.exp(s_scr[:, t * KC:(t + 1) * KC] - m)
            l = l + jnp.sum(p, axis=-1, keepdims=True)
            acc = acc + jnp.dot(p.astype(BF16), ckv[pl.ds(t * KC, KC), :], preferred_element_type=F32)
        cc = acc / l
        for g in range(DC // 128):
            cc_scr[g] = cc[:, g * 128:(g + 1) * 128]

    def stage_ctx(g):
        cc = cc_scr[g]
        acc = ctx_scr[...]
        for cl in range(128):
            acc = acc + cc[:, cl:cl + 1] * wuv[g * 128 + cl].astype(F32)
        ctx_scr[...] = acc

    def stage_head(h):
        q = q_scr[h].astype(BF16)
        s = jax.lax.dot_general(q, kb[h], (((1,), (1,)), ((), ())), preferred_element_type=F32) * SCALE
        m = jnp.max(s, axis=-1, keepdims=True)
        p = jnp.exp(s - m)
        l = jnp.sum(p, axis=-1, keepdims=True)
        o = jnp.dot(p.astype(BF16), vb[h], preferred_element_type=F32)
        o_scr[h] = o / l

    start(x_hbm, x_v, sem0.at[2], 0)
    start(gate_hbm, gate_v, sem1.at[2], 1)
    issue_p1(0)
    issue_p1(1)
    wait_all(x_v, sem0.at[2])
    wait_all(gate_v, sem1.at[2])

    xf = x_v[0].astype(F32)
    xb = jnp.broadcast_to(xf, (8, M)).astype(BF16)
    xcol[...] = jnp.broadcast_to(xf, (128, M)).T
    gsum = jnp.sum(xf * gate_v[...].astype(F32).reshape(1, M), axis=-1, keepdims=True)
    g = jax.nn.sigmoid(gsum)
    ctx_scr[...] = jnp.zeros_like(ctx_scr)

    static_steps = ([("p1", j) for j in range(N_P1)] + [("p2", j) for j in range(N_P2)]
                    + [("p3", j) for j in range(N_P3)])
    n_static = len(static_steps)

    def issue_step(s):
        if s < n_static:
            kind, j = static_steps[s]
            {"p1": issue_p1, "p2": issue_p2, "p3": issue_p3}[kind](j)
        else:
            issue_kv(s - n_static)

    for s, (kind, j) in enumerate(static_steps):
        issue_step(s + 2)
        if kind == "p1":
            wait_p1(j)
            stage_p1(j, xb)
            if j == N_P1 - 1:
                stage_q_finish()
        elif kind == "p2":
            wait_p2(j)
            stage_qabs(j)
        else:
            wait_p3(j)
            if j == 0:
                stage_a_scores()
            else:
                stage_a_softmax_pv()

    def head_body(h, c):
        @pl.when(h < H - 2)
        def _():
            issue_kv(h + 2)

        for j in range(2):
            @pl.when(h == H - 2 + j)
            def _(j=j):
                issue_p4(j)

        wait_all(kb.at[h], sem0.at[slot(PH + h)])
        wait_all(vb.at[h], sem1.at[slot(PH + h)])
        stage_head(h)

        @pl.when(h < DC // 128)
        def _():
            stage_ctx(h)
        return c
    jax.lax.fori_loop(0, H, head_body, 0)

    acc_a = jnp.zeros((8, M), F32)
    acc_b = jnp.zeros((8, M), F32)
    for j in range(N_P4):
        if j + 2 < N_P4:
            issue_p4(j + 2)
        for h0, nh, sl in p4_groups(j):
            wait_wo(h0, nh, sl)
            for h in range(h0, h0 + nh):
                ctx_h = jnp.broadcast_to(ctx_scr[h:h + 1, :], (8, D)).astype(BF16)
                acc_a = acc_a + jnp.dot(ctx_h, woa[h], preferred_element_type=F32)
                acc_b = acc_b + jnp.dot(o_scr[h].astype(BF16), wob[pl.ds(h * D, D), :],
                                        preferred_element_type=F32)

    out = g * acc_a[0:1, :] + (1.0 - g) * acc_b[0:1, :]
    o_ref[0] = out.astype(o_ref.dtype)


@jax.jit
def pallas_gated_mix__compressed_kv_cla__gqa_block_cached__decode_kernel(
    A_x: jax.Array,
    A_c_kv: jax.Array,
    A_w_q: jax.Array,
    A_w_uk: jax.Array,
    A_w_uv: jax.Array,
    A_w_o: jax.Array,
    B_x: jax.Array,
    B_k_cache: jax.Array,
    B_v_cache: jax.Array,
    B_wq: jax.Array,
    B_wo: jax.Array,
    gate_w: jax.Array,
):
    del B_x
    any_spec = pl.BlockSpec(memory_space=pl.ANY)
    dma = pltpu.SemaphoreType.DMA
    return pl.pallas_call(
        _kernel,
        out_shape=jax.ShapeDtypeStruct((1, 1, M), A_x.dtype),
        in_specs=[any_spec] * 11,
        out_specs=pl.BlockSpec(memory_space=pltpu.VMEM),
        scratch_shapes=[
            pltpu.VMEM((1, 1, M), BF16),
            pltpu.VMEM((M,), BF16),
            pltpu.VMEM((SK, DC), BF16),
            pltpu.VMEM((M, H, D), BF16),
            pltpu.VMEM((DC, H, D), BF16),
            pltpu.VMEM((DC, H, D), BF16),
            pltpu.VMEM((H, D, M), BF16),
            pltpu.VMEM((H, SK, D), BF16),
            pltpu.VMEM((H, SK, D), BF16),
            pltpu.VMEM((M, H * D), BF16),
            pltpu.VMEM((H * D, M), BF16),
            pltpu.VMEM((M, 128), F32),
            pltpu.VMEM((8, H * D), F32),
            pltpu.VMEM((H, 8, D), F32),
            pltpu.VMEM((H, D), F32),
            pltpu.VMEM((H, DC), F32),
            pltpu.VMEM((H, SK), F32),
            pltpu.VMEM((DC // 128, H, 128), F32),
            pltpu.VMEM((H, D), F32),
            pltpu.VMEM((H, 8, D), F32),
            dma((RING + len(LAST_SPLIT) - 1,)), dma((RING + len(LAST_SPLIT) - 1,)),
        ],
        compiler_params=pltpu.CompilerParams(vmem_limit_bytes=112 * 1024 * 1024),
    )(A_x, A_c_kv, A_w_q, A_w_uk, A_w_uv, A_w_o, B_k_cache, B_v_cache, B_wq, B_wo, gate_w)
```

```python
import jax
import jax.numpy as jnp
import jax.experimental.pallas as pl
import jax.experimental.pallas.tpu as pltpu

F32 = jnp.float32
BF16 = jnp.bfloat16

M = 640
H = 32
D = 128
DC = 512
SK = 4096
SCALE = D ** -0.5
RING = 3


def _kernel(
    x_hbm, ckv_hbm, wqa_hbm, wuk_hbm, wuv_hbm, woa_hbm, k_hbm, v_hbm, wqb_hbm, wob_hbm, gate_hbm,
    o_ref,
    x_v, gate_v, ckv, wqa, wuk, wuv, woa, kb, vb, wqb, wob,
    xcol, qb_acc, q_scr, qa_scr, r_scr, s_scr, cc_scr, ctx_scr, o_scr,
    sem0, sem1,
):
    sems = (sem0, sem1)

    def start(src, dst, queue, sl):
        pltpu.make_async_copy(src, dst, sems[queue].at[sl]).start(priority=queue)

    def wait_all(dst, queue, sl):
        pltpu.make_async_copy(dst, dst, sems[queue].at[sl]).wait()

    def slot(s):
        return s % RING if isinstance(s, int) else jax.lax.rem(s, RING)

    def rounds(j0, j1, streams, fn):
        def body(j, c):
            for s in range(streams):
                fn(s, j)
            return c
        jax.lax.fori_loop(j0, j1, body, 0)

    def d_wqb(i, sl):
        r = pl.multiple_of((i // 2) * 8, 8)
        c = pl.multiple_of((i % 2) * 2048, 128)
        start(wqb_hbm.at[pl.ds(r, 8), pl.ds(c, 2048)], wqb.at[pl.ds(r, 8), pl.ds(c, 2048)], 0, sl)

    def d_slab(src, dst, i, q, sl):
        start(src.at[pl.ds(i * 4, 4)], dst.at[pl.ds(i * 4, 4)], q, sl)

    def d_ckv(i, sl):
        r = pl.multiple_of(i * 32, 32)
        start(ckv_hbm.at[0, pl.ds(r, 32), :], ckv.at[pl.ds(r, 32), :], 1, sl)

    def d_kv(h, i, sl):
        r = pl.multiple_of(i * 128, 128)
        start(k_hbm.at[0, h, pl.ds(r, 128), :], kb.at[h, pl.ds(r, 128), :], 0, sl)
        start(v_hbm.at[0, h, pl.ds(r, 128), :], vb.at[h, pl.ds(r, 128), :], 1, sl)

    def d_wo(h, p, i, sl):
        r = pl.multiple_of(i * 32, 32)
        start(woa_hbm.at[h, pl.ds(r, 32), :], woa.at[p, pl.ds(r, 32), :], 0, sl)
        src_r = pl.multiple_of(h * D + r, 32)
        dst_r = pl.multiple_of(p * D + r, 32)
        start(wob_hbm.at[pl.ds(src_r, 32), :], wob.at[pl.ds(dst_r, 32), :], 1, sl)

    def win_q(r0, n):
        ns = n // 64

        def issue(part, sl):
            lo, hi = [(0, 8), (8, 16)][part] if ns <= 4 else [(0, 5), (5, 10), (10, 16)][part]

            def f(s, j):
                i = r0 // 4 + s * 16 + j
                d_wqb(i, sl)
                d_slab(wqa_hbm, wqa, i, 1, sl)
            rounds(lo, hi, ns, f)

        def wait(sl):
            wait_all(wqb.at[pl.ds(r0, n), :], 0, sl)
            wait_all(wqa.at[pl.ds(r0, n)], 1, sl)
        return issue, (2 if ns <= 4 else 3), wait

    def win_uk(t):
        def issue(part, sl):
            def f(s, j):
                i = t * 64 + s * 16 + j
                d_slab(wuk_hbm, wuk, i, 0, sl)
                d_ckv(i, sl)
            rounds(8 * part, 8 * part + 8, 4, f)

        def wait(sl):
            wait_all(wuk.at[pl.ds(t * 256, 256)], 0, sl)
            wait_all(ckv.at[pl.ds(t * 2048, 2048), :], 1, sl)
        return issue, 2, wait

    def win_uv():
        def issue(part, sl):
            def f(s, j):
                i = s * 16 + j
                d_slab(wuv_hbm, wuv, i, 0, sl)
                d_slab(wuv_hbm, wuv, 64 + i, 1, sl)
            rounds(8 * part, 8 * part + 8, 4, f)

        def wait(sl):
            wait_all(wuv.at[pl.ds(0, 256)], 0, sl)
            wait_all(wuv.at[pl.ds(256, 256)], 1, sl)
        return issue, 2, wait

    def win_kv(w):
        def issue(part, sl):
            def f(s, j):
                d_kv(2 * w + s // 2, (s % 2) * 16 + j, sl)
            lo = 8 * part if isinstance(part, int) else part * 8
            rounds(lo, lo + 8, 4, f)

        def wait(sl):
            wait_all(kb.at[pl.ds(2 * w, 2)], 0, sl)
            wait_all(vb.at[pl.ds(2 * w, 2)], 1, sl)
        return issue, 2, wait

    def wo_group(p0, round_heads):
        def issue(sl):
            p = p0
            for hs in round_heads:
                def f(s, j, hs=hs, p=p):
                    d_wo(hs[s], p + s, j, sl)
                rounds(0, 4, len(hs), f)
                p += len(hs)

        n = sum(len(hs) for hs in round_heads)

        def wait(sl):
            wait_all(woa.at[pl.ds(p0, n)], 0, sl)
            wait_all(wob.at[pl.ds(p0 * D, n * D), :], 1, sl)
        heads = [h for hs in round_heads for h in hs]
        return issue, wait, list(zip(range(p0, p0 + n), heads))

    def rnd(base, j):
        return [base + 4 * s + j for s in range(4)]

    def wo_window(p0, parts):
        groups, p = [], p0
        for round_heads in parts:
            groups.append(wo_group(p, round_heads))
            p += sum(len(hs) for hs in round_heads)
        n = p - p0

        def wait(sl):
            wait_all(woa.at[pl.ds(p0, n)], 0, sl)
            wait_all(wob.at[pl.ds(p0 * D, n * D), :], 1, sl)
        return (lambda part, sl: groups[part][0](sl)), wait, [x for grp in groups for x in grp[2]]

    wo_windows = [
        wo_window(0, [[rnd(0, 0), rnd(0, 1)], [rnd(0, 2), rnd(0, 3)]]),
        wo_window(16, [[rnd(16, 0), rnd(16, 1)]]),
        wo_window(24, [[rnd(16, 2)]]),
        wo_window(28, [[[19], [23]]]),
        wo_window(30, [[[27]]]),
        wo_window(31, [[[31]]]),
    ]

    def stage_qb(r0, n, xb):
        part = jnp.dot(xb[:, r0:r0 + n], wqb[pl.ds(r0, n), :], preferred_element_type=F32)
        if r0 == 0:
            qb_acc[...] = part
        else:
            part = part + qb_acc[...]
            for h in range(H):
                q_scr[h] = part[:, h * D:(h + 1) * D]

    def stage_qa(r0, n):
        unroll = 16

        def body(i, acc):
            for u in range(unroll):
                m = r0 + i * unroll + u
                acc = acc + xcol[pl.ds(m, 1), :] * wqa[m].astype(F32)
            return acc
        acc = jax.lax.fori_loop(0, n // unroll, body, jnp.zeros((H, D), F32))
        if r0 == 0:
            qa_scr[...] = acc
        else:
            qa_scr[...] += acc

    def stage_qabs(j):
        q = qa_scr[...]
        lane = jax.lax.broadcasted_iota(jnp.int32, (H, 128), 1)
        unroll = 16

        def body(i, r):
            for u in range(unroll):
                cl = i * unroll + u
                s = jnp.sum(wuk[j * 128 + cl].astype(F32) * q, axis=-1, keepdims=True)
                r = jnp.where(lane == cl, s, r)
            return r
        r_scr[:, j * 128:(j + 1) * 128] = jax.lax.fori_loop(
            0, 128 // unroll, body, jnp.zeros((H, 128), F32))

    KC = 1024

    def stage_a_scores():
        r = r_scr[...].astype(BF16)
        for t in range(SK // KC):
            s = jax.lax.dot_general(r, ckv[pl.ds(t * KC, KC), :], (((1,), (1,)), ((), ())),
                                    preferred_element_type=F32)
            s_scr[:, t * KC:(t + 1) * KC] = s * SCALE

    def stage_a_softmax_pv():
        m = s_scr[:, 0:KC]
        for t in range(1, SK // KC):
            m = jnp.maximum(m, s_scr[:, t * KC:(t + 1) * KC])
        m = jnp.max(m, axis=-1, keepdims=True)
        l = jnp.zeros((H, 1), F32)
        acc = jnp.zeros((H, DC), F32)
        for t in range(SK // KC):
            p = jnp.exp(s_scr[:, t * KC:(t + 1) * KC] - m)
            l = l + jnp.sum(p, axis=-1, keepdims=True)
            acc = acc + jnp.dot(p.astype(BF16), ckv[pl.ds(t * KC, KC), :], preferred_element_type=F32)
        cc = acc / l
        for g in range(DC // 128):
            cc_scr[g] = cc[:, g * 128:(g + 1) * 128]

    def stage_ctx(g):
        cc = cc_scr[g]
        acc = ctx_scr[...]
        for cl in range(128):
            acc = acc + cc[:, cl:cl + 1] * wuv[g * 128 + cl].astype(F32)
        ctx_scr[...] = acc

    def stage_head(h):
        q = q_scr[h].astype(BF16)
        s = jax.lax.dot_general(q, kb[h], (((1,), (1,)), ((), ())), preferred_element_type=F32) * SCALE
        m = jnp.max(s, axis=-1, keepdims=True)
        p = jnp.exp(s - m)
        l = jnp.sum(p, axis=-1, keepdims=True)
        o = jnp.dot(p.astype(BF16), vb[h], preferred_element_type=F32)
        o_scr[h] = o / l

    windows = [win_q(0, 256), win_q(256, 384), win_uk(0), win_uk(1), win_uv()]
    n_static = len(windows)

    start(x_hbm, x_v, 0, 2)
    start(gate_hbm, gate_v, 1, 2)
    for part in range(windows[0][1]):
        windows[0][0](part, slot(0))
    wait_all(x_v, 0, 2)
    wait_all(gate_v, 1, 2)

    xf = x_v[0].astype(F32)
    xb = jnp.broadcast_to(xf, (8, M)).astype(BF16)
    xcol[...] = jnp.broadcast_to(xf, (128, M)).T
    gsum = jnp.sum(xf * gate_v[...].astype(F32).reshape(1, M), axis=-1, keepdims=True)
    g = jax.nn.sigmoid(gsum)
    ctx_scr[...] = jnp.zeros_like(ctx_scr)

    pieces = [
        [lambda: stage_qb(0, 256, xb), lambda: stage_qa(0, 256)],
        [lambda: stage_qb(256, 384, xb), lambda: stage_qa(256, 384)],
        [lambda: stage_qabs(0), lambda: stage_qabs(1)],
        [lambda: stage_qabs(2), lambda: stage_qabs(3)],
        [stage_a_scores, stage_a_softmax_pv],
    ]
    NW = H // 2
    kv0, kv1 = win_kv(0), win_kv(1)

    def issue(win, parts, n):
        for part in parts:
            win[0](part, slot(n))

    static_issue = [
        (lambda: issue(windows[1], (0, 1), 1), lambda: issue(windows[1], (2,), 1)),
        (lambda: issue(windows[2], (0, 1), 2), lambda: issue(windows[3], (0,), 3)),
        (lambda: issue(windows[3], (1,), 3), lambda: issue(windows[4], (0,), 4)),
        (lambda: issue(windows[4], (1,), 4), lambda: issue(kv0, (0,), 5)),
        (lambda: issue(kv0, (1,), 5), lambda: issue(kv1, (0,), 6)),
    ]
    for n in range(n_static):
        static_issue[n][0]()
        windows[n][2](slot(n))
        pieces[n][0]()
        static_issue[n][1]()
        pieces[n][1]()

    n0 = n_static + NW

    def kv_body(w, c):
        n = n_static + w

        @pl.when(w < NW - 1)
        def _():
            win_kv(w + 1)[0](1, slot(n + 1))

        @pl.when(w == NW - 1)
        def _():
            wo_windows[0][0](1, slot(n0))

        win_kv(w)[2](slot(n))
        stage_head(2 * w)

        @pl.when(w < NW - 2)
        def _():
            win_kv(w + 2)[0](0, slot(n + 2))

        @pl.when(w == NW - 2)
        def _():
            wo_windows[0][0](0, slot(n0))

        @pl.when(w == NW - 1)
        def _():
            wo_windows[1][0](0, slot(n0 + 1))

        stage_head(2 * w + 1)

        @pl.when(w < DC // 128)
        def _():
            stage_ctx(w)
        return c
    jax.lax.fori_loop(0, NW, kv_body, 0)

    acc = [jnp.zeros((8, M), F32), jnp.zeros((8, M), F32)]

    def project(heads):
        for p, h in heads:
            ctx_h = jnp.broadcast_to(ctx_scr[h:h + 1, :], (8, D)).astype(BF16)
            acc[0] = acc[0] + jnp.dot(ctx_h, woa[p], preferred_element_type=F32)
            acc[1] = acc[1] + jnp.dot(o_scr[h].astype(BF16), wob[pl.ds(p * D, D), :],
                                      preferred_element_type=F32)

    def wo_issue(k):
        wo_windows[k][0](0, slot(n0 + k))

    def wo_wait(k):
        wo_windows[k][1](slot(n0 + k))

    wo_issue(2)
    wo_wait(0)
    project(wo_windows[0][2][:8])
    wo_issue(3)
    project(wo_windows[0][2][8:])
    wo_wait(1)
    wo_issue(4)
    project(wo_windows[1][2])
    wo_wait(2)
    wo_issue(5)
    project(wo_windows[2][2])
    for k in (3, 4, 5):
        wo_wait(k)
        project(wo_windows[k][2])
    acc_a, acc_b = acc

    out = g * acc_a[0:1, :] + (1.0 - g) * acc_b[0:1, :]
    o_ref[0] = out.astype(o_ref.dtype)


@jax.jit
def pallas_gated_mix__compressed_kv_cla__gqa_block_cached__decode_kernel(
    A_x: jax.Array,
    A_c_kv: jax.Array,
    A_w_q: jax.Array,
    A_w_uk: jax.Array,
    A_w_uv: jax.Array,
    A_w_o: jax.Array,
    B_x: jax.Array,
    B_k_cache: jax.Array,
    B_v_cache: jax.Array,
    B_wq: jax.Array,
    B_wo: jax.Array,
    gate_w: jax.Array,
):
    del B_x
    any_spec = pl.BlockSpec(memory_space=pl.ANY)
    return pl.pallas_call(
        _kernel,
        out_shape=jax.ShapeDtypeStruct((1, 1, M), A_x.dtype),
        in_specs=[any_spec] * 11,
        out_specs=pl.BlockSpec(memory_space=pltpu.VMEM),
        scratch_shapes=[
            pltpu.VMEM((1, 1, M), BF16),
            pltpu.VMEM((M,), BF16),
            pltpu.VMEM((SK, DC), BF16),
            pltpu.VMEM((M, H, D), BF16),
            pltpu.VMEM((DC, H, D), BF16),
            pltpu.VMEM((DC, H, D), BF16),
            pltpu.VMEM((H, D, M), BF16),
            pltpu.VMEM((H, SK, D), BF16),
            pltpu.VMEM((H, SK, D), BF16),
            pltpu.VMEM((M, H * D), BF16),
            pltpu.VMEM((H * D, M), BF16),
            pltpu.VMEM((M, 128), F32),
            pltpu.VMEM((8, H * D), F32),
            pltpu.VMEM((H, 8, D), F32),
            pltpu.VMEM((H, D), F32),
            pltpu.VMEM((H, DC), F32),
            pltpu.VMEM((H, SK), F32),
            pltpu.VMEM((DC // 128, H, 128), F32),
            pltpu.VMEM((H, D), F32),
            pltpu.VMEM((H, 8, D), F32),
            pltpu.SemaphoreType.DMA((RING,)),
            pltpu.SemaphoreType.DMA((RING,)),
        ],
        compiler_params=pltpu.CompilerParams(vmem_limit_bytes=112 * 1024 * 1024),
    )(A_x, A_c_kv, A_w_q, A_w_uk, A_w_uv, A_w_o, B_k_cache, B_v_cache, B_wq, B_wo, gate_w)
```

```python
import jax
import jax.numpy as jnp
import jax.experimental.pallas as pl
import jax.experimental.pallas.tpu as pltpu

F32 = jnp.float32
BF16 = jnp.bfloat16

M = 640
H = 32
D = 128
DC = 512
SK = 4096
SCALE = D ** -0.5
RING = 3

A_PHASE = 0
K_PHASE = 64
V_PHASE = 64


def _kernel(
    x_hbm, ckv_hbm, wqa_hbm, wuk_hbm, wuv_hbm, woa_hbm, k_hbm, v_hbm, wqb_hbm, wob_hbm, gate_hbm,
    o_ref,
    x_v, gate_v, ckv, wqa, wuk, wuv, woa, kb, vb, wqb, wob,
    xcol, qb_acc, q_scr, qa_scr, r_scr, s_scr, cc_scr, ctx_scr, o_scr,
    sem0, sem1,
):
    sems = (sem0, sem1)

    def start(src, dst, queue, sl):
        pltpu.make_async_copy(src, dst, sems[queue].at[sl]).start(priority=queue)

    def wait_all(dst, queue, sl):
        pltpu.make_async_copy(dst, dst, sems[queue].at[sl]).wait()

    def slot(s):
        return s % RING if isinstance(s, int) else jax.lax.rem(s, RING)

    def rounds(j0, j1, streams, fn):
        def body(j, c):
            for s in range(streams):
                fn(s, j)
            return c
        jax.lax.fori_loop(j0, j1, body, 0)

    def d_wqb(i, sl):
        r = pl.multiple_of((i // 2) * 8, 8)
        c = pl.multiple_of((i % 2) * 2048, 128)
        start(wqb_hbm.at[pl.ds(r, 8), pl.ds(c, 2048)], wqb.at[pl.ds(r, 8), pl.ds(c, 2048)], 0, sl)

    def d_slab(src, dst, u, n, q, sl):
        start(src.at[pl.ds(u, n)], dst.at[pl.ds(u, n)], q, sl)

    def d_ckv(u, n, sl):
        r = pl.multiple_of(u * 8, 8)
        start(ckv_hbm.at[0, pl.ds(r, n * 8), :], ckv.at[pl.ds(r, n * 8), :], 1, sl)

    def d_rows(src, dst, h, r, n, q, sl):
        start(src.at[0, h, pl.ds(r, n), :], dst.at[h, pl.ds(r, n), :], q, sl)

    def d_wo(h, p, i, sl):
        r = pl.multiple_of(i * 32, 32)
        start(woa_hbm.at[h, pl.ds(r, 32), :], woa.at[p, pl.ds(r, 32), :], 0, sl)
        src_r = pl.multiple_of(h * D + r, 32)
        dst_r = pl.multiple_of(p * D + r, 32)
        start(wob_hbm.at[pl.ds(src_r, 32), :], wob.at[pl.ds(dst_r, 32), :], 1, sl)

    def streams(u0, ns, parts, fns):
        def issue(part, sl):
            lo, hi = parts[part]
            last = hi == 16 and A_PHASE > 0
            if lo == 0 and A_PHASE:
                for fn in fns:
                    fn(u0, A_PHASE, sl)

            def f(s, j):
                for fn in fns:
                    fn(u0 + A_PHASE + s * 64 + j * 4, 4, sl)
            rounds(lo, hi - 1 if last else hi, ns, f)
            if last:
                for s in range(ns):
                    for fn in fns:
                        fn(u0 + A_PHASE + s * 64 + 60, 4 - A_PHASE if s == ns - 1 else 4, sl)
        return issue

    def u_wqb(u, n, sl):
        assert isinstance(n, int)
        if n == 4 and A_PHASE == 0:
            r = pl.multiple_of((u // 8) * 8, 8)
            c = pl.multiple_of((u % 8) * 512, 128)
            start(wqb_hbm.at[pl.ds(r, 8), pl.ds(c, 2048)], wqb.at[pl.ds(r, 8), pl.ds(c, 2048)], 0, sl)
        else:
            for k in range(0, n, 2):
                uu = u + k
                r = pl.multiple_of((uu // 8) * 8, 8)
                c = pl.multiple_of((uu % 8) * 512, 128)
                start(wqb_hbm.at[pl.ds(r, 8), pl.ds(c, 1024)], wqb.at[pl.ds(r, 8), pl.ds(c, 1024)], 0, sl)

    def win_q(r0, n):
        ns = n // 64
        parts = [(0, 8), (8, 16)] if ns <= 4 else [(0, 5), (5, 10), (10, 16)]
        issue = streams(r0, ns, parts, [
            u_wqb, lambda u, k, sl: d_slab(wqa_hbm, wqa, u, k, 1, sl)])

        def wait(sl):
            wait_all(wqb.at[pl.ds(r0, n), :], 0, sl)
            wait_all(wqa.at[pl.ds(r0, n)], 1, sl)
        return issue, len(parts), wait

    def win_uk(t):
        issue = streams(t * 256, 4, [(0, 8), (8, 16)], [
            lambda u, k, sl: d_slab(wuk_hbm, wuk, u, k, 0, sl), d_ckv])

        def wait(sl):
            wait_all(wuk.at[pl.ds(t * 256, 256)], 0, sl)
            wait_all(ckv.at[pl.ds(t * 2048, 2048), :], 1, sl)
        return issue, 2, wait

    def win_uv():
        issue = streams(0, 4, [(0, 8), (8, 16)], [
            lambda u, k, sl: d_slab(wuv_hbm, wuv, u, k, 0, sl),
            lambda u, k, sl: d_slab(wuv_hbm, wuv, 256 + u, k, 1, sl)])

        def wait(sl):
            wait_all(wuv.at[pl.ds(0, 256)], 0, sl)
            wait_all(wuv.at[pl.ds(256, 256)], 1, sl)
        return issue, 2, wait

    def win_kv(w):
        arrays = ((k_hbm, kb, K_PHASE, 0), (v_hbm, vb, V_PHASE, 1))

        def rnd_full(s, j, sl):
            h = 2 * w + s // 2
            for src, dst, ph, q in arrays:
                r = pl.multiple_of(ph + ((s % 2) * 16 + j) * 128, 64 if ph else 128)
                d_rows(src, dst, h, r, 128, q, sl)

        def issue(part, sl):
            shifted = any(a[2] for a in arrays)
            if part == 0:
                if shifted:
                    for hh in range(2):
                        for src, dst, ph, q in arrays:
                            if ph:
                                d_rows(src, dst, 2 * w + hh, 0, ph, q, sl)
                rounds(0, 8, 4, lambda s, j: rnd_full(s, j, sl))
            elif not shifted:
                rounds(8, 16, 4, lambda s, j: rnd_full(s, j, sl))
            else:
                rounds(8, 15, 4, lambda s, j: rnd_full(s, j, sl))
                for s in range(4):
                    h = 2 * w + s // 2
                    for src, dst, ph, q in arrays:
                        r = ph + ((s % 2) * 16 + 15) * 128
                        d_rows(src, dst, h, r, min(128, SK - r), q, sl)

        def wait(sl):
            wait_all(kb.at[pl.ds(2 * w, 2)], 0, sl)
            wait_all(vb.at[pl.ds(2 * w, 2)], 1, sl)
        return issue, 2, wait

    def wo_group(p0, round_heads):
        def issue(sl):
            p = p0
            for hs in round_heads:
                def f(s, j, hs=hs, p=p):
                    d_wo(hs[s], p + s, j, sl)
                rounds(0, 4, len(hs), f)
                p += len(hs)

        n = sum(len(hs) for hs in round_heads)

        def wait(sl):
            wait_all(woa.at[pl.ds(p0, n)], 0, sl)
            wait_all(wob.at[pl.ds(p0 * D, n * D), :], 1, sl)
        heads = [h for hs in round_heads for h in hs]
        return issue, wait, list(zip(range(p0, p0 + n), heads))

    def rnd(base, j):
        return [base + 4 * s + j for s in range(4)]

    def wo_window(p0, parts):
        groups, p = [], p0
        for round_heads in parts:
            groups.append(wo_group(p, round_heads))
            p += sum(len(hs) for hs in round_heads)
        n = p - p0

        def wait(sl):
            wait_all(woa.at[pl.ds(p0, n)], 0, sl)
            wait_all(wob.at[pl.ds(p0 * D, n * D), :], 1, sl)
        return (lambda part, sl: groups[part][0](sl)), wait, [x for grp in groups for x in grp[2]]

    wo_windows = [
        wo_window(0, [[rnd(0, 0), rnd(0, 1)], [rnd(0, 2), rnd(0, 3)]]),
        wo_window(16, [[rnd(16, 0), rnd(16, 1)]]),
        wo_window(24, [[rnd(16, 2)]]),
        wo_window(28, [[[19], [23]]]),
        wo_window(30, [[[27]]]),
        wo_window(31, [[[31]]]),
    ]

    def stage_qb(r0, n, xb):
        part = jnp.dot(xb[:, r0:r0 + n], wqb[pl.ds(r0, n), :], preferred_element_type=F32)
        if r0 == 0:
            qb_acc[...] = part
        else:
            part = part + qb_acc[...]
            for h in range(H):
                q_scr[h] = part[:, h * D:(h + 1) * D]

    def stage_qa(r0, n):
        unroll = 16

        def body(i, acc):
            for u in range(unroll):
                m = r0 + i * unroll + u
                acc = acc + xcol[pl.ds(m, 1), :] * wqa[m].astype(F32)
            return acc
        acc = jax.lax.fori_loop(0, n // unroll, body, jnp.zeros((H, D), F32))
        if r0 == 0:
            qa_scr[...] = acc
        else:
            qa_scr[...] += acc

    def stage_qabs(j):
        q = qa_scr[...]
        lane = jax.lax.broadcasted_iota(jnp.int32, (H, 128), 1)
        unroll = 16

        def body(i, r):
            for u in range(unroll):
                cl = i * unroll + u
                s = jnp.sum(wuk[j * 128 + cl].astype(F32) * q, axis=-1, keepdims=True)
                r = jnp.where(lane == cl, s, r)
            return r
        r_scr[:, j * 128:(j + 1) * 128] = jax.lax.fori_loop(
            0, 128 // unroll, body, jnp.zeros((H, 128), F32))

    KC = 1024

    def stage_a_scores():
        r = r_scr[...].astype(BF16)
        for t in range(SK // KC):
            s = jax.lax.dot_general(r, ckv[pl.ds(t * KC, KC), :], (((1,), (1,)), ((), ())),
                                    preferred_element_type=F32)
            s_scr[:, t * KC:(t + 1) * KC] = s * SCALE

    def stage_a_softmax_pv():
        m = s_scr[:, 0:KC]
        for t in range(1, SK // KC):
            m = jnp.maximum(m, s_scr[:, t * KC:(t + 1) * KC])
        m = jnp.max(m, axis=-1, keepdims=True)
        l = jnp.zeros((H, 1), F32)
        acc = jnp.zeros((H, DC), F32)
        for t in range(SK // KC):
            p = jnp.exp(s_scr[:, t * KC:(t + 1) * KC] - m)
            l = l + jnp.sum(p, axis=-1, keepdims=True)
            acc = acc + jnp.dot(p.astype(BF16), ckv[pl.ds(t * KC, KC), :], preferred_element_type=F32)
        cc = acc / l
        for g in range(DC // 128):
            cc_scr[g] = cc[:, g * 128:(g + 1) * 128]

    def stage_ctx(g):
        cc = cc_scr[g]
        acc = ctx_scr[...]
        for cl in range(128):
            acc = acc + cc[:, cl:cl + 1] * wuv[g * 128 + cl].astype(F32)
        ctx_scr[...] = acc

    def stage_head(h):
        q = q_scr[h].astype(BF16)
        s = jax.lax.dot_general(q, kb[h], (((1,), (1,)), ((), ())), preferred_element_type=F32) * SCALE
        m = jnp.max(s, axis=-1, keepdims=True)
        p = jnp.exp(s - m)
        l = jnp.sum(p, axis=-1, keepdims=True)
        o = jnp.dot(p.astype(BF16), vb[h], preferred_element_type=F32)
        o_scr[h] = o / l

    windows = [win_q(0, 256), win_q(256, 384), win_uk(0), win_uk(1), win_uv()]
    n_static = len(windows)

    start(x_hbm, x_v, 0, 2)
    start(gate_hbm, gate_v, 1, 2)
    for part in range(windows[0][1]):
        windows[0][0](part, slot(0))
    wait_all(x_v, 0, 2)
    wait_all(gate_v, 1, 2)

    xf = x_v[0].astype(F32)
    xb = jnp.broadcast_to(xf, (8, M)).astype(BF16)
    xcol[...] = jnp.broadcast_to(xf, (128, M)).T
    gsum = jnp.sum(xf * gate_v[...].astype(F32).reshape(1, M), axis=-1, keepdims=True)
    g = jax.nn.sigmoid(gsum)
    ctx_scr[...] = jnp.zeros_like(ctx_scr)

    pieces = [
        [lambda: stage_qb(0, 256, xb), lambda: stage_qa(0, 256)],
        [lambda: stage_qb(256, 384, xb), lambda: stage_qa(256, 384)],
        [lambda: stage_qabs(0), lambda: stage_qabs(1)],
        [lambda: stage_qabs(2), lambda: stage_qabs(3)],
        [stage_a_scores, stage_a_softmax_pv],
    ]
    NW = H // 2
    kv0, kv1 = win_kv(0), win_kv(1)

    def issue(win, parts, n):
        for part in parts:
            win[0](part, slot(n))

    static_issue = [
        (lambda: issue(windows[1], (0, 1), 1), lambda: issue(windows[1], (2,), 1)),
        (lambda: issue(windows[2], (0, 1), 2), lambda: issue(windows[3], (0,), 3)),
        (lambda: issue(windows[3], (1,), 3), lambda: issue(windows[4], (0,), 4)),
        (lambda: issue(windows[4], (1,), 4), lambda: issue(kv0, (0,), 5)),
        (lambda: issue(kv0, (1,), 5), lambda: issue(kv1, (0,), 6)),
    ]
    for n in range(n_static):
        static_issue[n][0]()
        windows[n][2](slot(n))
        pieces[n][0]()
        static_issue[n][1]()
        pieces[n][1]()

    n0 = n_static + NW

    def kv_body(w, c):
        n = n_static + w

        @pl.when(w < NW - 1)
        def _():
            win_kv(w + 1)[0](1, slot(n + 1))

        @pl.when(w == NW - 1)
        def _():
            wo_windows[0][0](1, slot(n0))

        win_kv(w)[2](slot(n))
        stage_head(2 * w)

        @pl.when(w < NW - 2)
        def _():
            win_kv(w + 2)[0](0, slot(n + 2))

        @pl.when(w == NW - 2)
        def _():
            wo_windows[0][0](0, slot(n0))

        @pl.when(w == NW - 1)
        def _():
            wo_windows[1][0](0, slot(n0 + 1))

        stage_head(2 * w + 1)

        @pl.when(w < DC // 128)
        def _():
            stage_ctx(w)
        return c
    jax.lax.fori_loop(0, NW, kv_body, 0)

    acc = [jnp.zeros((8, M), F32), jnp.zeros((8, M), F32)]

    def project(heads):
        for p, h in heads:
            ctx_h = jnp.broadcast_to(ctx_scr[h:h + 1, :], (8, D)).astype(BF16)
            acc[0] = acc[0] + jnp.dot(ctx_h, woa[p], preferred_element_type=F32)
            acc[1] = acc[1] + jnp.dot(o_scr[h].astype(BF16), wob[pl.ds(p * D, D), :],
                                      preferred_element_type=F32)

    def wo_issue(k):
        wo_windows[k][0](0, slot(n0 + k))

    def wo_wait(k):
        wo_windows[k][1](slot(n0 + k))

    wo_issue(2)
    wo_wait(0)
    project(wo_windows[0][2][:8])
    wo_issue(3)
    project(wo_windows[0][2][8:])
    wo_wait(1)
    wo_issue(4)
    project(wo_windows[1][2])
    wo_wait(2)
    wo_issue(5)
    project(wo_windows[2][2])
    for k in (3, 4, 5):
        wo_wait(k)
        project(wo_windows[k][2])
    acc_a, acc_b = acc

    out = g * acc_a[0:1, :] + (1.0 - g) * acc_b[0:1, :]
    o_ref[0] = out.astype(o_ref.dtype)


@jax.jit
def pallas_gated_mix__compressed_kv_cla__gqa_block_cached__decode_kernel(
    A_x: jax.Array,
    A_c_kv: jax.Array,
    A_w_q: jax.Array,
    A_w_uk: jax.Array,
    A_w_uv: jax.Array,
    A_w_o: jax.Array,
    B_x: jax.Array,
    B_k_cache: jax.Array,
    B_v_cache: jax.Array,
    B_wq: jax.Array,
    B_wo: jax.Array,
    gate_w: jax.Array,
):
    del B_x
    any_spec = pl.BlockSpec(memory_space=pl.ANY)
    return pl.pallas_call(
        _kernel,
        out_shape=jax.ShapeDtypeStruct((1, 1, M), A_x.dtype),
        in_specs=[any_spec] * 11,
        out_specs=pl.BlockSpec(memory_space=pltpu.VMEM),
        scratch_shapes=[
            pltpu.VMEM((1, 1, M), BF16),
            pltpu.VMEM((M,), BF16),
            pltpu.VMEM((SK, DC), BF16),
            pltpu.VMEM((M, H, D), BF16),
            pltpu.VMEM((DC, H, D), BF16),
            pltpu.VMEM((DC, H, D), BF16),
            pltpu.VMEM((H, D, M), BF16),
            pltpu.VMEM((H, SK, D), BF16),
            pltpu.VMEM((H, SK, D), BF16),
            pltpu.VMEM((M, H * D), BF16),
            pltpu.VMEM((H * D, M), BF16),
            pltpu.VMEM((M, 128), F32),
            pltpu.VMEM((8, H * D), F32),
            pltpu.VMEM((H, 8, D), F32),
            pltpu.VMEM((H, D), F32),
            pltpu.VMEM((H, DC), F32),
            pltpu.VMEM((H, SK), F32),
            pltpu.VMEM((DC // 128, H, 128), F32),
            pltpu.VMEM((H, D), F32),
            pltpu.VMEM((H, 8, D), F32),
            pltpu.SemaphoreType.DMA((RING,)),
            pltpu.SemaphoreType.DMA((RING,)),
        ],
        compiler_params=pltpu.CompilerParams(vmem_limit_bytes=112 * 1024 * 1024),
    )(A_x, A_c_kv, A_w_q, A_w_uk, A_w_uv, A_w_o, B_k_cache, B_v_cache, B_wq, B_wo, gate_w)
```

```python
import jax
import jax.numpy as jnp
import jax.experimental.pallas as pl
import jax.experimental.pallas.tpu as pltpu

F32 = jnp.float32
BF16 = jnp.bfloat16

M = 640
H = 32
D = 128
DC = 512
SK = 4096
SCALE = D ** -0.5
RING = 3

A_PHASE = 0
K_PHASE = 64
V_PHASE = 64


def _kernel(
    x_hbm, ckv_hbm, wqa_hbm, wuk_hbm, wuv_hbm, woa_hbm, k_hbm, v_hbm, wqb_hbm, wob_hbm, gate_hbm,
    o_ref,
    x_v, gate_v, ckv, wqa, wuk, wuv, woa, kb, vb, wqb, wob,
    xcol, qb_acc, q_scr, qa_scr, r_scr, s_scr, cc_scr, ctx_scr, o_scr,
    sem0, sem1,
):
    sems = (sem0, sem1)

    def start(src, dst, queue, sl):
        pltpu.make_async_copy(src, dst, sems[queue].at[sl]).start(priority=queue)

    def wait_all(dst, queue, sl):
        pltpu.make_async_copy(dst, dst, sems[queue].at[sl]).wait()

    def slot(s):
        return s % RING if isinstance(s, int) else jax.lax.rem(s, RING)

    def rounds(j0, j1, streams, fn):
        def body(j, c):
            for s in range(streams):
                fn(s, j)
            return c
        jax.lax.fori_loop(j0, j1, body, 0)

    def d_wqb(i, sl):
        r = pl.multiple_of((i // 2) * 8, 8)
        c = pl.multiple_of((i % 2) * 2048, 128)
        start(wqb_hbm.at[pl.ds(r, 8), pl.ds(c, 2048)], wqb.at[pl.ds(r, 8), pl.ds(c, 2048)], 0, sl)

    def d_slab(src, dst, u, n, q, sl):
        start(src.at[pl.ds(u, n)], dst.at[pl.ds(u, n)], q, sl)

    def d_ckv(u, n, sl):
        r = pl.multiple_of(u * 8, 8)
        start(ckv_hbm.at[0, pl.ds(r, n * 8), :], ckv.at[pl.ds(r, n * 8), :], 1, sl)

    def d_rows(src, dst, h, r, n, q, sl):
        start(src.at[0, h, pl.ds(r, n), :], dst.at[h, pl.ds(r, n), :], q, sl)

    def d_woa(h, p, i, sl):
        r = pl.multiple_of(i * 32, 32)
        start(woa_hbm.at[h, pl.ds(r, 32), :], woa.at[p, pl.ds(r, 32), :], 0, sl)

    def d_wob(h, p, i, sl):
        src_r = pl.multiple_of(h * D + i * 32, 32)
        dst_r = pl.multiple_of(p * D + i * 32, 32)
        start(wob_hbm.at[pl.ds(src_r, 32), :], wob.at[pl.ds(dst_r, 32), :], 1, sl)

    def streams(u0, ns, parts, fns):
        def issue(part, sl):
            lo, hi = parts[part]
            last = hi == 16 and A_PHASE > 0
            if lo == 0 and A_PHASE:
                for fn in fns:
                    fn(u0, A_PHASE, sl)

            def f(s, j):
                for fn in fns:
                    fn(u0 + A_PHASE + s * 64 + j * 4, 4, sl)
            rounds(lo, hi - 1 if last else hi, ns, f)
            if last:
                for s in range(ns):
                    for fn in fns:
                        fn(u0 + A_PHASE + s * 64 + 60, 4 - A_PHASE if s == ns - 1 else 4, sl)
        return issue

    def u_wqb(u, n, sl):
        assert isinstance(n, int)
        if n == 4 and A_PHASE == 0:
            r = pl.multiple_of((u // 8) * 8, 8)
            c = pl.multiple_of((u % 8) * 512, 128)
            start(wqb_hbm.at[pl.ds(r, 8), pl.ds(c, 2048)], wqb.at[pl.ds(r, 8), pl.ds(c, 2048)], 0, sl)
        else:
            for k in range(0, n, 2):
                uu = u + k
                r = pl.multiple_of((uu // 8) * 8, 8)
                c = pl.multiple_of((uu % 8) * 512, 128)
                start(wqb_hbm.at[pl.ds(r, 8), pl.ds(c, 1024)], wqb.at[pl.ds(r, 8), pl.ds(c, 1024)], 0, sl)

    def win_q(r0, n):
        ns = n // 64
        parts = [(0, 8), (8, 16)] if ns <= 4 else [(0, 5), (5, 10), (10, 16)]
        issue = streams(r0, ns, parts, [
            u_wqb, lambda u, k, sl: d_slab(wqa_hbm, wqa, u, k, 1, sl)])

        def wait(sl):
            wait_all(wqb.at[pl.ds(r0, n), :], 0, sl)
            wait_all(wqa.at[pl.ds(r0, n)], 1, sl)
        return issue, len(parts), wait

    def win_uk(t):
        issue = streams(t * 256, 4, [(0, 8), (8, 16)], [
            lambda u, k, sl: d_slab(wuk_hbm, wuk, u, k, 0, sl), d_ckv])

        def wait(sl):
            wait_all(wuk.at[pl.ds(t * 256, 256)], 0, sl)
            wait_all(ckv.at[pl.ds(t * 2048, 2048), :], 1, sl)
        return issue, 2, wait

    def win_uv():
        issue = streams(0, 4, [(0, 8), (8, 16)], [
            lambda u, k, sl: d_slab(wuv_hbm, wuv, u, k, 0, sl),
            lambda u, k, sl: d_slab(wuv_hbm, wuv, 256 + u, k, 1, sl)])

        def wait(sl):
            wait_all(wuv.at[pl.ds(0, 256)], 0, sl)
            wait_all(wuv.at[pl.ds(256, 256)], 1, sl)
        return issue, 2, wait

    def win_kv(w):
        arrays = ((k_hbm, kb, K_PHASE, 0), (v_hbm, vb, V_PHASE, 1))

        def rnd_full(s, j, sl):
            h = 2 * w + s // 2
            for src, dst, ph, q in arrays:
                r = pl.multiple_of(ph + ((s % 2) * 16 + j) * 128, 64 if ph else 128)
                d_rows(src, dst, h, r, 128, q, sl)

        def issue(part, sl):
            shifted = any(a[2] for a in arrays)
            if part == 0:
                if shifted:
                    for hh in range(2):
                        for src, dst, ph, q in arrays:
                            if ph:
                                d_rows(src, dst, 2 * w + hh, 0, ph, q, sl)
                rounds(0, 8, 4, lambda s, j: rnd_full(s, j, sl))
            elif not shifted:
                rounds(8, 16, 4, lambda s, j: rnd_full(s, j, sl))
            else:
                rounds(8, 15, 4, lambda s, j: rnd_full(s, j, sl))
                for s in range(4):
                    h = 2 * w + s // 2
                    for src, dst, ph, q in arrays:
                        r = ph + ((s % 2) * 16 + 15) * 128
                        d_rows(src, dst, h, r, min(128, SK - r), q, sl)

        def wait(sl):
            wait_all(kb.at[pl.ds(2 * w, 2)], 0, sl)
            wait_all(vb.at[pl.ds(2 * w, 2)], 1, sl)
        return issue, 2, wait

    wo_pos = [0, 0]

    def wo_window(parts):
        pa0, pb0 = wo_pos
        plan, heads_a, heads_b = [], [], []
        for part in parts:
            rs = []
            for ha, hb in part:
                rs.append(([(h, wo_pos[0] + n) for n, h in enumerate(ha)],
                           [(h, wo_pos[1] + n) for n, h in enumerate(hb)]))
                heads_a += rs[-1][0]
                heads_b += rs[-1][1]
                wo_pos[0] += len(ha)
                wo_pos[1] += len(hb)
            plan.append(rs)
        na, nb = wo_pos[0] - pa0, wo_pos[1] - pb0

        def issue(part, sl):
            for ra, rb in plan[part]:
                def f(s, j, ra=ra, rb=rb):
                    if s < len(ra):
                        d_woa(ra[s][0], ra[s][1], j, sl)
                    if s < len(rb):
                        d_wob(rb[s][0], rb[s][1], j, sl)
                rounds(0, 4, max(len(ra), len(rb)), f)

        def wait(sl):
            if na:
                wait_all(woa.at[pl.ds(pa0, na)], 0, sl)
            if nb:
                wait_all(wob.at[pl.ds(pb0 * D, nb * D), :], 1, sl)
        return issue, wait, heads_a, heads_b

    def rnd(base, j):
        hs = [base + 4 * s + j for s in range(4)]
        return hs, hs

    wo_windows = [
        wo_window([[rnd(0, 0), rnd(0, 1)], [rnd(0, 2), rnd(0, 3)]]),
        wo_window([[rnd(16, 0), rnd(16, 1)]]),
        wo_window([[rnd(16, 2)]]),
        wo_window([[([19], [19]), ([23], [23])]]),
        wo_window([[([27], [27]), ([31], [])]]),
        wo_window([[([], [31])]]),
    ]

    def stage_qb(r0, n, xb):
        part = jnp.dot(xb[:, r0:r0 + n], wqb[pl.ds(r0, n), :], preferred_element_type=F32)
        if r0 == 0:
            qb_acc[...] = part
        else:
            part = part + qb_acc[...]
            for h in range(H):
                q_scr[h] = part[:, h * D:(h + 1) * D]

    def stage_qa(r0, n):
        unroll = 16

        def body(i, acc):
            for u in range(unroll):
                m = r0 + i * unroll + u
                acc = acc + xcol[pl.ds(m, 1), :] * wqa[m].astype(F32)
            return acc
        acc = jax.lax.fori_loop(0, n // unroll, body, jnp.zeros((H, D), F32))
        if r0 == 0:
            qa_scr[...] = acc
        else:
            qa_scr[...] += acc

    def stage_qabs(j):
        q = qa_scr[...]
        lane = jax.lax.broadcasted_iota(jnp.int32, (H, 128), 1)
        unroll = 16

        def body(i, r):
            for u in range(unroll):
                cl = i * unroll + u
                s = jnp.sum(wuk[j * 128 + cl].astype(F32) * q, axis=-1, keepdims=True)
                r = jnp.where(lane == cl, s, r)
            return r
        r_scr[:, j * 128:(j + 1) * 128] = jax.lax.fori_loop(
            0, 128 // unroll, body, jnp.zeros((H, 128), F32))

    KC = 1024

    def stage_a_scores():
        r = r_scr[...].astype(BF16)
        for t in range(SK // KC):
            s = jax.lax.dot_general(r, ckv[pl.ds(t * KC, KC), :], (((1,), (1,)), ((), ())),
                                    preferred_element_type=F32)
            s_scr[:, t * KC:(t + 1) * KC] = s * SCALE

    def stage_a_softmax_pv():
        m = s_scr[:, 0:KC]
        for t in range(1, SK // KC):
            m = jnp.maximum(m, s_scr[:, t * KC:(t + 1) * KC])
        m = jnp.max(m, axis=-1, keepdims=True)
        l = jnp.zeros((H, 1), F32)
        acc = jnp.zeros((H, DC), F32)
        for t in range(SK // KC):
            p = jnp.exp(s_scr[:, t * KC:(t + 1) * KC] - m)
            l = l + jnp.sum(p, axis=-1, keepdims=True)
            acc = acc + jnp.dot(p.astype(BF16), ckv[pl.ds(t * KC, KC), :], preferred_element_type=F32)
        cc = acc / l
        for g in range(DC // 128):
            cc_scr[g] = cc[:, g * 128:(g + 1) * 128]

    def stage_ctx(g):
        cc = cc_scr[g]
        acc = ctx_scr[...]
        for cl in range(128):
            acc = acc + cc[:, cl:cl + 1] * wuv[g * 128 + cl].astype(F32)
        ctx_scr[...] = acc

    def stage_head(h):
        q = q_scr[h].astype(BF16)
        s = jax.lax.dot_general(q, kb[h], (((1,), (1,)), ((), ())), preferred_element_type=F32) * SCALE
        m = jnp.max(s, axis=-1, keepdims=True)
        p = jnp.exp(s - m)
        l = jnp.sum(p, axis=-1, keepdims=True)
        o = jnp.dot(p.astype(BF16), vb[h], preferred_element_type=F32)
        o_scr[h] = o / l

    windows = [win_q(0, 256), win_q(256, 384), win_uk(0), win_uk(1), win_uv()]
    n_static = len(windows)

    start(x_hbm, x_v, 0, 2)
    start(gate_hbm, gate_v, 1, 2)
    for part in range(windows[0][1]):
        windows[0][0](part, slot(0))
    wait_all(x_v, 0, 2)
    wait_all(gate_v, 1, 2)

    xf = x_v[0].astype(F32)
    xb = jnp.broadcast_to(xf, (8, M)).astype(BF16)
    xcol[...] = jnp.broadcast_to(xf, (128, M)).T
    gsum = jnp.sum(xf * gate_v[...].astype(F32).reshape(1, M), axis=-1, keepdims=True)
    g = jax.nn.sigmoid(gsum)
    ctx_scr[...] = jnp.zeros_like(ctx_scr)

    pieces = [
        [lambda: stage_qb(0, 256, xb), lambda: stage_qa(0, 256)],
        [lambda: stage_qb(256, 384, xb), lambda: stage_qa(256, 384)],
        [lambda: stage_qabs(0), lambda: stage_qabs(1)],
        [lambda: stage_qabs(2), lambda: stage_qabs(3)],
        [stage_a_scores, stage_a_softmax_pv],
    ]
    NW = H // 2
    kv0, kv1 = win_kv(0), win_kv(1)

    def issue(win, parts, n):
        for part in parts:
            win[0](part, slot(n))

    static_issue = [
        (lambda: issue(windows[1], (0, 1), 1), lambda: issue(windows[1], (2,), 1)),
        (lambda: issue(windows[2], (0, 1), 2), lambda: issue(windows[3], (0,), 3)),
        (lambda: issue(windows[3], (1,), 3), lambda: issue(windows[4], (0,), 4)),
        (lambda: issue(windows[4], (1,), 4), lambda: issue(kv0, (0,), 5)),
        (lambda: issue(kv0, (1,), 5), lambda: issue(kv1, (0,), 6)),
    ]
    for n in range(n_static):
        static_issue[n][0]()
        windows[n][2](slot(n))
        pieces[n][0]()
        static_issue[n][1]()
        pieces[n][1]()

    n0 = n_static + NW

    def kv_body(w, c):
        n = n_static + w

        @pl.when(w < NW - 1)
        def _():
            win_kv(w + 1)[0](1, slot(n + 1))

        @pl.when(w == NW - 1)
        def _():
            wo_windows[0][0](1, slot(n0))

        win_kv(w)[2](slot(n))
        stage_head(2 * w)

        @pl.when(w < NW - 2)
        def _():
            win_kv(w + 2)[0](0, slot(n + 2))

        @pl.when(w == NW - 2)
        def _():
            wo_windows[0][0](0, slot(n0))

        @pl.when(w == NW - 1)
        def _():
            wo_windows[1][0](0, slot(n0 + 1))

        stage_head(2 * w + 1)

        @pl.when(w < DC // 128)
        def _():
            stage_ctx(w)
        return c
    jax.lax.fori_loop(0, NW, kv_body, 0)

    acc = [jnp.zeros((8, M), F32), jnp.zeros((8, M), F32)]

    def project(k, lo=0, hi=None):
        _, _, heads_a, heads_b = wo_windows[k]
        for n in range(lo, max(len(heads_a), len(heads_b)) if hi is None else hi):
            if n < len(heads_a):
                h, p = heads_a[n]
                ctx_h = jnp.broadcast_to(ctx_scr[h:h + 1, :], (8, D)).astype(BF16)
                acc[0] = acc[0] + jnp.dot(ctx_h, woa[p], preferred_element_type=F32)
            if n < len(heads_b):
                h, p = heads_b[n]
                acc[1] = acc[1] + jnp.dot(o_scr[h].astype(BF16), wob[pl.ds(p * D, D), :],
                                          preferred_element_type=F32)

    def wo_issue(k):
        wo_windows[k][0](0, slot(n0 + k))

    def wo_wait(k):
        wo_windows[k][1](slot(n0 + k))

    wo_issue(2)
    wo_wait(0)
    project(0, 0, 8)
    wo_issue(3)
    project(0, 8, 16)
    wo_wait(1)
    wo_issue(4)
    project(1)
    wo_wait(2)
    wo_issue(5)
    project(2)
    for k in (3, 4, 5):
        wo_wait(k)
        project(k)
    acc_a, acc_b = acc

    out = g * acc_a[0:1, :] + (1.0 - g) * acc_b[0:1, :]
    o_ref[0] = out.astype(o_ref.dtype)


@jax.jit
def pallas_gated_mix__compressed_kv_cla__gqa_block_cached__decode_kernel(
    A_x: jax.Array,
    A_c_kv: jax.Array,
    A_w_q: jax.Array,
    A_w_uk: jax.Array,
    A_w_uv: jax.Array,
    A_w_o: jax.Array,
    B_x: jax.Array,
    B_k_cache: jax.Array,
    B_v_cache: jax.Array,
    B_wq: jax.Array,
    B_wo: jax.Array,
    gate_w: jax.Array,
):
    del B_x
    any_spec = pl.BlockSpec(memory_space=pl.ANY)
    return pl.pallas_call(
        _kernel,
        out_shape=jax.ShapeDtypeStruct((1, 1, M), A_x.dtype),
        in_specs=[any_spec] * 11,
        out_specs=pl.BlockSpec(memory_space=pltpu.VMEM),
        scratch_shapes=[
            pltpu.VMEM((1, 1, M), BF16),
            pltpu.VMEM((M,), BF16),
            pltpu.VMEM((SK, DC), BF16),
            pltpu.VMEM((M, H, D), BF16),
            pltpu.VMEM((DC, H, D), BF16),
            pltpu.VMEM((DC, H, D), BF16),
            pltpu.VMEM((H, D, M), BF16),
            pltpu.VMEM((H, SK, D), BF16),
            pltpu.VMEM((H, SK, D), BF16),
            pltpu.VMEM((M, H * D), BF16),
            pltpu.VMEM((H * D, M), BF16),
            pltpu.VMEM((M, 128), F32),
            pltpu.VMEM((8, H * D), F32),
            pltpu.VMEM((H, 8, D), F32),
            pltpu.VMEM((H, D), F32),
            pltpu.VMEM((H, DC), F32),
            pltpu.VMEM((H, SK), F32),
            pltpu.VMEM((DC // 128, H, 128), F32),
            pltpu.VMEM((H, D), F32),
            pltpu.VMEM((H, 8, D), F32),
            pltpu.SemaphoreType.DMA((RING,)),
            pltpu.SemaphoreType.DMA((RING,)),
        ],
        compiler_params=pltpu.CompilerParams(vmem_limit_bytes=112 * 1024 * 1024),
    )(A_x, A_c_kv, A_w_q, A_w_uk, A_w_uv, A_w_o, B_k_cache, B_v_cache, B_wq, B_wo, gate_w)
```

```python
import jax
import jax.numpy as jnp
import jax.experimental.pallas as pl
import jax.experimental.pallas.tpu as pltpu

F32 = jnp.float32
BF16 = jnp.bfloat16

M = 640
H = 32
D = 128
DC = 512
SK = 4096
SCALE = D ** -0.5
RING = 3

KV_PHASE = 64


def _kernel(
    x_hbm, ckv_hbm, wqa_hbm, wuk_hbm, wuv_hbm, woa_hbm, k_hbm, v_hbm, wqb_hbm, wob_hbm, gate_hbm,
    o_ref,
    x_v, gate_v, ckv, wqa, wuk, wuv, woa, kb, vb, wqb, wob,
    xcol, qb_acc, q_scr, qa_scr, r_scr, s_scr, cc_scr, ctx_scr, o_scr,
    sem0, sem1,
):
    sems = (sem0, sem1)

    def start(src, dst, queue, sl):
        pltpu.make_async_copy(src, dst, sems[queue].at[sl]).start(priority=queue)

    def wait_all(dst, queue, sl):
        pltpu.make_async_copy(dst, dst, sems[queue].at[sl]).wait()

    def slot(s):
        return s % RING if isinstance(s, int) else jax.lax.rem(s, RING)

    def rounds(j0, j1, streams, fn):
        def body(j, c):
            for s in range(streams):
                fn(s, j)
            return c
        jax.lax.fori_loop(j0, j1, body, 0)

    def d_wqb(u, sl):
        r = pl.multiple_of((u // 8) * 8, 8)
        c = pl.multiple_of((u % 8) * 512, 128)
        start(wqb_hbm.at[pl.ds(r, 8), pl.ds(c, 2048)], wqb.at[pl.ds(r, 8), pl.ds(c, 2048)], 0, sl)

    def d_slab(src, dst, u, q, sl):
        start(src.at[pl.ds(u, 4)], dst.at[pl.ds(u, 4)], q, sl)

    def d_ckv(u, sl):
        r = pl.multiple_of(u * 8, 8)
        start(ckv_hbm.at[0, pl.ds(r, 32), :], ckv.at[pl.ds(r, 32), :], 1, sl)

    def d_rows(src, dst, h, r, n, q, sl):
        start(src.at[0, h, pl.ds(r, n), :], dst.at[h, pl.ds(r, n), :], q, sl)

    def d_woa(h, p, i, sl):
        r = pl.multiple_of(i * 32, 32)
        start(woa_hbm.at[h, pl.ds(r, 32), :], woa.at[p, pl.ds(r, 32), :], 0, sl)

    def d_wob(h, p, i, sl):
        src_r = pl.multiple_of(h * D + i * 32, 32)
        dst_r = pl.multiple_of(p * D + i * 32, 32)
        start(wob_hbm.at[pl.ds(src_r, 32), :], wob.at[pl.ds(dst_r, 32), :], 1, sl)

    def streams(u0, ns, parts, fns):
        def issue(part, sl):
            def f(s, j):
                for fn in fns:
                    fn(u0 + s * 64 + j * 4, sl)
            rounds(parts[part][0], parts[part][1], ns, f)
        return issue

    def win_q(r0, n):
        ns = n // 64
        parts = [(0, 8), (8, 16)] if ns <= 4 else [(0, 5), (5, 10), (10, 16)]
        issue = streams(r0, ns, parts, [d_wqb, lambda u, sl: d_slab(wqa_hbm, wqa, u, 1, sl)])

        def wait(sl):
            wait_all(wqb.at[pl.ds(r0, n), :], 0, sl)
            wait_all(wqa.at[pl.ds(r0, n)], 1, sl)
        return issue, len(parts), wait

    def win_uk(t):
        issue = streams(t * 256, 4, [(0, 8), (8, 16)],
                        [lambda u, sl: d_slab(wuk_hbm, wuk, u, 0, sl), d_ckv])

        def wait(sl):
            wait_all(wuk.at[pl.ds(t * 256, 256)], 0, sl)
            wait_all(ckv.at[pl.ds(t * 2048, 2048), :], 1, sl)
        return issue, 2, wait

    def win_uv():
        issue = streams(0, 4, [(0, 8), (8, 16)],
                        [lambda u, sl: d_slab(wuv_hbm, wuv, u, 0, sl),
                         lambda u, sl: d_slab(wuv_hbm, wuv, 256 + u, 1, sl)])

        def wait(sl):
            wait_all(wuv.at[pl.ds(0, 256)], 0, sl)
            wait_all(wuv.at[pl.ds(256, 256)], 1, sl)
        return issue, 2, wait

    def win_kv(w):
        def pair(s, r, n, sl):
            d_rows(k_hbm, kb, 2 * w + s // 2, r, n, 0, sl)
            d_rows(v_hbm, vb, 2 * w + s // 2, r, n, 1, sl)

        def full(s, j, sl):
            pair(s, pl.multiple_of(KV_PHASE + ((s % 2) * 16 + j) * 128, 16), 128, sl)

        def issue(part, sl):
            if part == 0:
                if KV_PHASE:
                    for s in (0, 2):
                        pair(s, 0, KV_PHASE, sl)
                rounds(0, 8, 4, lambda s, j: full(s, j, sl))
            else:
                rounds(8, 15, 4, lambda s, j: full(s, j, sl))
                for s in range(4):
                    r = KV_PHASE + ((s % 2) * 16 + 15) * 128
                    pair(s, r, min(128, SK - r), sl)

        def wait(sl):
            wait_all(kb.at[pl.ds(2 * w, 2)], 0, sl)
            wait_all(vb.at[pl.ds(2 * w, 2)], 1, sl)
        return issue, 2, wait

    wo_pos = [0, 0]

    def wo_window(parts):
        pa0, pb0 = wo_pos
        plan, heads_a, heads_b = [], [], []
        for part in parts:
            rs = []
            for ha, hb in part:
                rs.append(([(h, wo_pos[0] + n) for n, h in enumerate(ha)],
                           [(h, wo_pos[1] + n) for n, h in enumerate(hb)]))
                heads_a += rs[-1][0]
                heads_b += rs[-1][1]
                wo_pos[0] += len(ha)
                wo_pos[1] += len(hb)
            plan.append(rs)
        na, nb = wo_pos[0] - pa0, wo_pos[1] - pb0

        def issue(part, sl):
            for ra, rb in plan[part]:
                def f(s, j, ra=ra, rb=rb):
                    if s < len(ra):
                        d_woa(ra[s][0], ra[s][1], j, sl)
                    if s < len(rb):
                        d_wob(rb[s][0], rb[s][1], j, sl)
                rounds(0, 4, max(len(ra), len(rb)), f)

        def wait(sl):
            if na:
                wait_all(woa.at[pl.ds(pa0, na)], 0, sl)
            if nb:
                wait_all(wob.at[pl.ds(pb0 * D, nb * D), :], 1, sl)
        return issue, wait, heads_a, heads_b

    def rnd(base, j):
        hs = [base + 4 * s + j for s in range(4)]
        return hs, hs

    wo_windows = [
        wo_window([[rnd(0, 0), rnd(0, 1)], [rnd(0, 2), rnd(0, 3)]]),
        wo_window([[rnd(16, 0), rnd(16, 1)]]),
        wo_window([[rnd(16, 2)]]),
        wo_window([[([19], [19]), ([23], [23])]]),
        wo_window([[([27], [27]), ([31], [])]]),
        wo_window([[([], [31])]]),
    ]

    def stage_qb(r0, n, xb):
        part = jnp.dot(xb[:, r0:r0 + n], wqb[pl.ds(r0, n), :], preferred_element_type=F32)
        if r0 == 0:
            qb_acc[...] = part
        else:
            part = part + qb_acc[...]
            for h in range(H):
                q_scr[h] = part[:, h * D:(h + 1) * D]

    def stage_qa(r0, n):
        unroll = 16

        def body(i, acc):
            for u in range(unroll):
                m = r0 + i * unroll + u
                acc = acc + xcol[pl.ds(m, 1), :] * wqa[m].astype(F32)
            return acc
        acc = jax.lax.fori_loop(0, n // unroll, body, jnp.zeros((H, D), F32))
        if r0 == 0:
            qa_scr[...] = acc
        else:
            qa_scr[...] += acc

    def stage_qabs(j):
        q = qa_scr[...]
        lane = jax.lax.broadcasted_iota(jnp.int32, (H, 128), 1)
        unroll = 16

        def body(i, r):
            for u in range(unroll):
                cl = i * unroll + u
                s = jnp.sum(wuk[j * 128 + cl].astype(F32) * q, axis=-1, keepdims=True)
                r = jnp.where(lane == cl, s, r)
            return r
        r_scr[:, j * 128:(j + 1) * 128] = jax.lax.fori_loop(
            0, 128 // unroll, body, jnp.zeros((H, 128), F32))

    KC = 1024

    def stage_a_scores():
        r = r_scr[...].astype(BF16)
        for t in range(SK // KC):
            s = jax.lax.dot_general(r, ckv[pl.ds(t * KC, KC), :], (((1,), (1,)), ((), ())),
                                    preferred_element_type=F32)
            s_scr[:, t * KC:(t + 1) * KC] = s * SCALE

    def stage_a_softmax_pv():
        m = s_scr[:, 0:KC]
        for t in range(1, SK // KC):
            m = jnp.maximum(m, s_scr[:, t * KC:(t + 1) * KC])
        m = jnp.max(m, axis=-1, keepdims=True)
        l = jnp.zeros((H, 1), F32)
        acc = jnp.zeros((H, DC), F32)
        for t in range(SK // KC):
            p = jnp.exp(s_scr[:, t * KC:(t + 1) * KC] - m)
            l = l + jnp.sum(p, axis=-1, keepdims=True)
            acc = acc + jnp.dot(p.astype(BF16), ckv[pl.ds(t * KC, KC), :], preferred_element_type=F32)
        cc = acc / l
        for g in range(DC // 128):
            cc_scr[g] = cc[:, g * 128:(g + 1) * 128]

    def stage_ctx(g):
        cc = cc_scr[g]
        acc = ctx_scr[...]
        for cl in range(128):
            acc = acc + cc[:, cl:cl + 1] * wuv[g * 128 + cl].astype(F32)
        ctx_scr[...] = acc

    def stage_head(h):
        q = q_scr[h].astype(BF16)
        s = jax.lax.dot_general(q, kb[h], (((1,), (1,)), ((), ())), preferred_element_type=F32) * SCALE
        m = jnp.max(s, axis=-1, keepdims=True)
        p = jnp.exp(s - m)
        l = jnp.sum(p, axis=-1, keepdims=True)
        o = jnp.dot(p.astype(BF16), vb[h], preferred_element_type=F32)
        o_scr[h] = o / l

    windows = [win_q(0, 256), win_q(256, 384), win_uk(0), win_uk(1), win_uv()]
    n_static = len(windows)

    start(x_hbm, x_v, 0, 2)
    start(gate_hbm, gate_v, 1, 2)
    for part in range(windows[0][1]):
        windows[0][0](part, slot(0))
    wait_all(x_v, 0, 2)
    wait_all(gate_v, 1, 2)

    xf = x_v[0].astype(F32)
    xb = jnp.broadcast_to(xf, (8, M)).astype(BF16)
    xcol[...] = jnp.broadcast_to(xf, (128, M)).T
    gsum = jnp.sum(xf * gate_v[...].astype(F32).reshape(1, M), axis=-1, keepdims=True)
    g = jax.nn.sigmoid(gsum)
    ctx_scr[...] = jnp.zeros_like(ctx_scr)

    pieces = [
        [lambda: stage_qb(0, 256, xb), lambda: stage_qa(0, 256)],
        [lambda: stage_qb(256, 384, xb), lambda: stage_qa(256, 384)],
        [lambda: stage_qabs(0), lambda: stage_qabs(1)],
        [lambda: stage_qabs(2), lambda: stage_qabs(3)],
        [stage_a_scores, stage_a_softmax_pv],
    ]
    NW = H // 2
    kv0, kv1 = win_kv(0), win_kv(1)

    def issue(win, parts, n):
        for part in parts:
            win[0](part, slot(n))

    static_issue = [
        (lambda: issue(windows[1], (0, 1), 1), lambda: issue(windows[1], (2,), 1)),
        (lambda: issue(windows[2], (0, 1), 2), lambda: issue(windows[3], (0,), 3)),
        (lambda: issue(windows[3], (1,), 3), lambda: issue(windows[4], (0,), 4)),
        (lambda: issue(windows[4], (1,), 4), lambda: issue(kv0, (0,), 5)),
        (lambda: issue(kv0, (1,), 5), lambda: issue(kv1, (0,), 6)),
    ]
    for n in range(n_static):
        static_issue[n][0]()
        windows[n][2](slot(n))
        pieces[n][0]()
        static_issue[n][1]()
        pieces[n][1]()

    n0 = n_static + NW

    def kv_body(w, c):
        n = n_static + w

        @pl.when(w < NW - 1)
        def _():
            win_kv(w + 1)[0](1, slot(n + 1))

        @pl.when(w == NW - 1)
        def _():
            wo_windows[0][0](1, slot(n0))

        win_kv(w)[2](slot(n))
        stage_head(2 * w)

        @pl.when(w < NW - 2)
        def _():
            win_kv(w + 2)[0](0, slot(n + 2))

        @pl.when(w == NW - 2)
        def _():
            wo_windows[0][0](0, slot(n0))

        @pl.when(w == NW - 1)
        def _():
            wo_windows[1][0](0, slot(n0 + 1))

        stage_head(2 * w + 1)

        @pl.when(w < DC // 128)
        def _():
            stage_ctx(w)
        return c
    jax.lax.fori_loop(0, NW, kv_body, 0)

    acc = [jnp.zeros((8, M), F32), jnp.zeros((8, M), F32)]

    def project(k, lo=0, hi=None):
        _, _, heads_a, heads_b = wo_windows[k]
        for n in range(lo, max(len(heads_a), len(heads_b)) if hi is None else hi):
            if n < len(heads_a):
                h, p = heads_a[n]
                ctx_h = jnp.broadcast_to(ctx_scr[h:h + 1, :], (8, D)).astype(BF16)
                acc[0] = acc[0] + jnp.dot(ctx_h, woa[p], preferred_element_type=F32)
            if n < len(heads_b):
                h, p = heads_b[n]
                acc[1] = acc[1] + jnp.dot(o_scr[h].astype(BF16), wob[pl.ds(p * D, D), :],
                                          preferred_element_type=F32)

    def wo_issue(k):
        wo_windows[k][0](0, slot(n0 + k))

    def wo_wait(k):
        wo_windows[k][1](slot(n0 + k))

    wo_issue(2)
    wo_wait(0)
    project(0, 0, 8)
    wo_issue(3)
    project(0, 8, 16)
    wo_wait(1)
    wo_issue(4)
    project(1)
    wo_wait(2)
    wo_issue(5)
    project(2)
    for k in (3, 4, 5):
        wo_wait(k)
        project(k)
    acc_a, acc_b = acc

    out = g * acc_a[0:1, :] + (1.0 - g) * acc_b[0:1, :]
    o_ref[0] = out.astype(o_ref.dtype)


@jax.jit
def pallas_gated_mix__compressed_kv_cla__gqa_block_cached__decode_kernel(
    A_x: jax.Array,
    A_c_kv: jax.Array,
    A_w_q: jax.Array,
    A_w_uk: jax.Array,
    A_w_uv: jax.Array,
    A_w_o: jax.Array,
    B_x: jax.Array,
    B_k_cache: jax.Array,
    B_v_cache: jax.Array,
    B_wq: jax.Array,
    B_wo: jax.Array,
    gate_w: jax.Array,
):
    del B_x
    any_spec = pl.BlockSpec(memory_space=pl.ANY)
    return pl.pallas_call(
        _kernel,
        out_shape=jax.ShapeDtypeStruct((1, 1, M), A_x.dtype),
        in_specs=[any_spec] * 11,
        out_specs=pl.BlockSpec(memory_space=pltpu.VMEM),
        scratch_shapes=[
            pltpu.VMEM((1, 1, M), BF16),
            pltpu.VMEM((M,), BF16),
            pltpu.VMEM((SK, DC), BF16),
            pltpu.VMEM((M, H, D), BF16),
            pltpu.VMEM((DC, H, D), BF16),
            pltpu.VMEM((DC, H, D), BF16),
            pltpu.VMEM((H, D, M), BF16),
            pltpu.VMEM((H, SK, D), BF16),
            pltpu.VMEM((H, SK, D), BF16),
            pltpu.VMEM((M, H * D), BF16),
            pltpu.VMEM((H * D, M), BF16),
            pltpu.VMEM((M, 128), F32),
            pltpu.VMEM((8, H * D), F32),
            pltpu.VMEM((H, 8, D), F32),
            pltpu.VMEM((H, D), F32),
            pltpu.VMEM((H, DC), F32),
            pltpu.VMEM((H, SK), F32),
            pltpu.VMEM((DC // 128, H, 128), F32),
            pltpu.VMEM((H, D), F32),
            pltpu.VMEM((H, 8, D), F32),
            pltpu.SemaphoreType.DMA((RING,)),
            pltpu.SemaphoreType.DMA((RING,)),
        ],
        compiler_params=pltpu.CompilerParams(vmem_limit_bytes=112 * 1024 * 1024),
    )(A_x, A_c_kv, A_w_q, A_w_uk, A_w_uv, A_w_o, B_k_cache, B_v_cache, B_wq, B_wo, gate_w)
```

```python
import jax
import jax.numpy as jnp
import jax.experimental.pallas as pl
import jax.experimental.pallas.tpu as pltpu

F32 = jnp.float32
BF16 = jnp.bfloat16

M = 640
H = 32
D = 128
DC = 512
SK = 4096
SCALE = D ** -0.5
RING = 3

KV_PHASE = 64


def _kernel(
    x_hbm, ckv_hbm, wqa_hbm, wuk_hbm, wuv_hbm, woa_hbm, k_hbm, v_hbm, wqb_hbm, wob_hbm, gate_hbm,
    o_ref,
    x_v, gate_v, ckv, wqa, wuk, wuv, woa, kb, vb, wqb, wob,
    xcol, qb_acc, q_scr, qa_scr, r_scr, s_scr, cc_scr, ctx_scr, o_scr,
    sem0, sem1,
):
    sems = (sem0, sem1)

    def start(src, dst, queue, sl):
        pltpu.make_async_copy(src, dst, sems[queue].at[sl]).start(priority=queue)

    def wait_all(dst, queue, sl):
        pltpu.make_async_copy(dst, dst, sems[queue].at[sl]).wait()

    def slot(s):
        return s % RING if isinstance(s, int) else jax.lax.rem(s, RING)

    def rounds(j0, j1, streams, fn):
        def body(j, c):
            for s in range(streams):
                fn(s, j)
            return c
        jax.lax.fori_loop(j0, j1, body, 0)

    def d_wqb(u, sl):
        r = pl.multiple_of((u // 8) * 8, 8)
        c = pl.multiple_of((u % 8) * 512, 128)
        start(wqb_hbm.at[pl.ds(r, 8), pl.ds(c, 2048)], wqb.at[pl.ds(r, 8), pl.ds(c, 2048)], 0, sl)

    def d_slab(src, dst, u, q, sl):
        start(src.at[pl.ds(u, 4)], dst.at[pl.ds(u, 4)], q, sl)

    def d_ckv(u, sl):
        r = pl.multiple_of(u * 8, 8)
        start(ckv_hbm.at[0, pl.ds(r, 32), :], ckv.at[pl.ds(r, 32), :], 1, sl)

    def d_kv(r, n, sl):
        start(k_hbm.at[pl.ds(r, n), :], kb.at[pl.ds(r, n), :], 0, sl)
        start(v_hbm.at[pl.ds(r, n), :], vb.at[pl.ds(r, n), :], 1, sl)

    def d_woa(h, p, i, sl):
        r = pl.multiple_of(i * 32, 32)
        start(woa_hbm.at[h, pl.ds(r, 32), :], woa.at[p, pl.ds(r, 32), :], 0, sl)

    def d_wob(h, p, i, sl):
        src_r = pl.multiple_of(h * D + i * 32, 32)
        dst_r = pl.multiple_of(p * D + i * 32, 32)
        start(wob_hbm.at[pl.ds(src_r, 32), :], wob.at[pl.ds(dst_r, 32), :], 1, sl)

    def streams(u0, ns, parts, fns):
        def issue(part, sl):
            def f(s, j):
                for fn in fns:
                    fn(u0 + s * 64 + j * 4, sl)
            rounds(parts[part][0], parts[part][1], ns, f)
        return issue

    def win_q(r0, n):
        ns = n // 64
        parts = [(0, 8), (8, 16)] if ns <= 4 else [(0, 5), (5, 10), (10, 16)]
        issue = streams(r0, ns, parts, [d_wqb, lambda u, sl: d_slab(wqa_hbm, wqa, u, 1, sl)])

        def wait(sl):
            wait_all(wqb.at[pl.ds(r0, n), :], 0, sl)
            wait_all(wqa.at[pl.ds(r0, n)], 1, sl)
        return issue, len(parts), wait

    def win_uk(t):
        issue = streams(t * 256, 4, [(0, 8), (8, 16)],
                        [lambda u, sl: d_slab(wuk_hbm, wuk, u, 0, sl), d_ckv])

        def wait(sl):
            wait_all(wuk.at[pl.ds(t * 256, 256)], 0, sl)
            wait_all(ckv.at[pl.ds(t * 2048, 2048), :], 1, sl)
        return issue, 2, wait

    def win_uv():
        issue = streams(0, 4, [(0, 8), (8, 16)],
                        [lambda u, sl: d_slab(wuv_hbm, wuv, u, 0, sl),
                         lambda u, sl: d_slab(wuv_hbm, wuv, 256 + u, 1, sl)])

        def wait(sl):
            wait_all(wuv.at[pl.ds(0, 256)], 0, sl)
            wait_all(wuv.at[pl.ds(256, 256)], 1, sl)
        return issue, 2, wait

    def win_kv(w):
        r0 = KV_PHASE + 2 * w * SK

        def full(s, j, sl):
            d_kv(pl.multiple_of(r0 + (s * 16 + j) * 128, 16), 128, sl)

        def issue(part, sl, first=False, last=False):
            if part == 0:
                if first and KV_PHASE:
                    d_kv(0, KV_PHASE, sl)
                rounds(0, 8, 4, lambda s, j: full(s, j, sl))
            elif last and KV_PHASE:
                rounds(8, 15, 4, lambda s, j: full(s, j, sl))
                for s in range(4):
                    d_kv(pl.multiple_of(r0 + (s * 16 + 15) * 128, 16),
                         128 - KV_PHASE if s == 3 else 128, sl)
            else:
                rounds(8, 16, 4, lambda s, j: full(s, j, sl))

        def wait(sl, first=False, last=False):
            lo = 0 if first else r0
            n = 2 * SK + (KV_PHASE if first else 0) - (KV_PHASE if last else 0)
            lo = lo if first else pl.multiple_of(lo, 16)
            wait_all(kb.at[pl.ds(lo, n), :], 0, sl)
            wait_all(vb.at[pl.ds(lo, n), :], 1, sl)
        return issue, 2, wait

    wo_pos = [0, 0]

    def wo_window(parts):
        pa0, pb0 = wo_pos
        plan, heads_a, heads_b = [], [], []
        for part in parts:
            rs = []
            for ha, hb in part:
                rs.append(([(h, wo_pos[0] + n) for n, h in enumerate(ha)],
                           [(h, wo_pos[1] + n) for n, h in enumerate(hb)]))
                heads_a += rs[-1][0]
                heads_b += rs[-1][1]
                wo_pos[0] += len(ha)
                wo_pos[1] += len(hb)
            plan.append(rs)
        na, nb = wo_pos[0] - pa0, wo_pos[1] - pb0

        def issue(part, sl):
            for ra, rb in plan[part]:
                def f(s, j, ra=ra, rb=rb):
                    if s < len(ra):
                        d_woa(ra[s][0], ra[s][1], j, sl)
                    if s < len(rb):
                        d_wob(rb[s][0], rb[s][1], j, sl)
                rounds(0, 4, max(len(ra), len(rb)), f)

        def wait(sl):
            if na:
                wait_all(woa.at[pl.ds(pa0, na)], 0, sl)
            if nb:
                wait_all(wob.at[pl.ds(pb0 * D, nb * D), :], 1, sl)
        return issue, wait, heads_a, heads_b

    def rnd(base, j):
        hs = [base + 4 * s + j for s in range(4)]
        return hs, hs

    wo_windows = [
        wo_window([[rnd(0, 0), rnd(0, 1)], [rnd(0, 2), rnd(0, 3)]]),
        wo_window([[rnd(16, 0), rnd(16, 1)]]),
        wo_window([[rnd(16, 2)]]),
        wo_window([[([19], [19]), ([23], [23])]]),
        wo_window([[([27], [27]), ([31], [])]]),
        wo_window([[([], [31])]]),
    ]

    def stage_qb(r0, n, xb):
        part = jnp.dot(xb[:, r0:r0 + n], wqb[pl.ds(r0, n), :], preferred_element_type=F32)
        if r0 == 0:
            qb_acc[...] = part
        else:
            part = part + qb_acc[...]
            for h in range(H):
                q_scr[h] = part[:, h * D:(h + 1) * D]

    def stage_qa(r0, n):
        unroll = 16

        def body(i, acc):
            for u in range(unroll):
                m = r0 + i * unroll + u
                acc = acc + xcol[pl.ds(m, 1), :] * wqa[m].astype(F32)
            return acc
        acc = jax.lax.fori_loop(0, n // unroll, body, jnp.zeros((H, D), F32))
        if r0 == 0:
            qa_scr[...] = acc
        else:
            qa_scr[...] += acc

    def stage_qabs(j):
        q = qa_scr[...]
        lane = jax.lax.broadcasted_iota(jnp.int32, (H, 128), 1)
        unroll = 16

        def body(i, r):
            for u in range(unroll):
                cl = i * unroll + u
                s = jnp.sum(wuk[j * 128 + cl].astype(F32) * q, axis=-1, keepdims=True)
                r = jnp.where(lane == cl, s, r)
            return r
        r_scr[:, j * 128:(j + 1) * 128] = jax.lax.fori_loop(
            0, 128 // unroll, body, jnp.zeros((H, 128), F32))

    KC = 1024

    def stage_a_scores():
        r = r_scr[...].astype(BF16)
        for t in range(SK // KC):
            s = jax.lax.dot_general(r, ckv[pl.ds(t * KC, KC), :], (((1,), (1,)), ((), ())),
                                    preferred_element_type=F32)
            s_scr[:, t * KC:(t + 1) * KC] = s * SCALE

    def stage_a_softmax_pv():
        m = s_scr[:, 0:KC]
        for t in range(1, SK // KC):
            m = jnp.maximum(m, s_scr[:, t * KC:(t + 1) * KC])
        m = jnp.max(m, axis=-1, keepdims=True)
        l = jnp.zeros((H, 1), F32)
        acc = jnp.zeros((H, DC), F32)
        for t in range(SK // KC):
            p = jnp.exp(s_scr[:, t * KC:(t + 1) * KC] - m)
            l = l + jnp.sum(p, axis=-1, keepdims=True)
            acc = acc + jnp.dot(p.astype(BF16), ckv[pl.ds(t * KC, KC), :], preferred_element_type=F32)
        cc = acc / l
        for g in range(DC // 128):
            cc_scr[g] = cc[:, g * 128:(g + 1) * 128]

    def stage_ctx(g):
        cc = cc_scr[g]
        acc = ctx_scr[...]
        for cl in range(128):
            acc = acc + cc[:, cl:cl + 1] * wuv[g * 128 + cl].astype(F32)
        ctx_scr[...] = acc

    def stage_head(h):
        q = q_scr[h].astype(BF16)
        r = pl.multiple_of(h * SK, SK)
        s = jax.lax.dot_general(q, kb[pl.ds(r, SK), :], (((1,), (1,)), ((), ())),
                                preferred_element_type=F32) * SCALE
        m = jnp.max(s, axis=-1, keepdims=True)
        p = jnp.exp(s - m)
        l = jnp.sum(p, axis=-1, keepdims=True)
        o = jnp.dot(p.astype(BF16), vb[pl.ds(r, SK), :], preferred_element_type=F32)
        o_scr[h] = o / l

    windows = [win_q(0, 256), win_q(256, 384), win_uk(0), win_uk(1), win_uv()]
    n_static = len(windows)

    start(x_hbm, x_v, 0, 2)
    start(gate_hbm, gate_v, 1, 2)
    for part in range(windows[0][1]):
        windows[0][0](part, slot(0))
    wait_all(x_v, 0, 2)
    wait_all(gate_v, 1, 2)

    xf = x_v[0].astype(F32)
    xb = jnp.broadcast_to(xf, (8, M)).astype(BF16)
    xcol[...] = jnp.broadcast_to(xf, (128, M)).T
    gsum = jnp.sum(xf * gate_v[...].astype(F32).reshape(1, M), axis=-1, keepdims=True)
    g = jax.nn.sigmoid(gsum)
    ctx_scr[...] = jnp.zeros_like(ctx_scr)

    pieces = [
        [lambda: stage_qb(0, 256, xb), lambda: stage_qa(0, 256)],
        [lambda: stage_qb(256, 384, xb), lambda: stage_qa(256, 384)],
        [lambda: stage_qabs(0), lambda: stage_qabs(1)],
        [lambda: stage_qabs(2), lambda: stage_qabs(3)],
        [stage_a_scores, stage_a_softmax_pv],
    ]
    NW = H // 2
    kv0, kv1 = win_kv(0), win_kv(1)

    def issue(win, parts, n):
        for part in parts:
            win[0](part, slot(n))

    static_issue = [
        (lambda: issue(windows[1], (0, 1), 1), lambda: issue(windows[1], (2,), 1)),
        (lambda: issue(windows[2], (0, 1), 2), lambda: issue(windows[3], (0,), 3)),
        (lambda: issue(windows[3], (1,), 3), lambda: issue(windows[4], (0,), 4)),
        (lambda: issue(windows[4], (1,), 4), lambda: kv0[0](0, slot(5), first=True)),
        (lambda: issue(kv0, (1,), 5), lambda: issue(kv1, (0,), 6)),
    ]
    for n in range(n_static):
        static_issue[n][0]()
        windows[n][2](slot(n))
        pieces[n][0]()
        static_issue[n][1]()
        pieces[n][1]()

    n0 = n_static + NW

    def kv_body(w, c):
        n = n_static + w

        @pl.when(w < NW - 2)
        def _():
            win_kv(w + 1)[0](1, slot(n + 1))

        @pl.when(w == NW - 2)
        def _():
            win_kv(NW - 1)[0](1, slot(n_static + NW - 1), last=True)

        @pl.when(w == NW - 1)
        def _():
            wo_windows[0][0](1, slot(n0))

        @pl.when(w == 0)
        def _():
            win_kv(0)[2](slot(n_static), first=True)

        @pl.when(jnp.logical_and(w > 0, w < NW - 1))
        def _():
            win_kv(w)[2](slot(n))

        @pl.when(w == NW - 1)
        def _():
            win_kv(NW - 1)[2](slot(n_static + NW - 1), last=True)

        stage_head(2 * w)

        @pl.when(w < NW - 2)
        def _():
            win_kv(w + 2)[0](0, slot(n + 2))

        @pl.when(w == NW - 2)
        def _():
            wo_windows[0][0](0, slot(n0))

        @pl.when(w == NW - 1)
        def _():
            wo_windows[1][0](0, slot(n0 + 1))

        stage_head(2 * w + 1)

        @pl.when(w < DC // 128)
        def _():
            stage_ctx(w)
        return c
    jax.lax.fori_loop(0, NW, kv_body, 0)

    acc = [jnp.zeros((8, M), F32), jnp.zeros((8, M), F32)]

    def project(k, lo=0, hi=None):
        _, _, heads_a, heads_b = wo_windows[k]
        for n in range(lo, max(len(heads_a), len(heads_b)) if hi is None else hi):
            if n < len(heads_a):
                h, p = heads_a[n]
                ctx_h = jnp.broadcast_to(ctx_scr[h:h + 1, :], (8, D)).astype(BF16)
                acc[0] = acc[0] + jnp.dot(ctx_h, woa[p], preferred_element_type=F32)
            if n < len(heads_b):
                h, p = heads_b[n]
                acc[1] = acc[1] + jnp.dot(o_scr[h].astype(BF16), wob[pl.ds(p * D, D), :],
                                          preferred_element_type=F32)

    def wo_issue(k):
        wo_windows[k][0](0, slot(n0 + k))

    def wo_wait(k):
        wo_windows[k][1](slot(n0 + k))

    wo_issue(2)
    wo_wait(0)
    project(0, 0, 8)
    wo_issue(3)
    project(0, 8, 16)
    wo_wait(1)
    wo_issue(4)
    project(1)
    wo_wait(2)
    wo_issue(5)
    project(2)
    for k in (3, 4, 5):
        wo_wait(k)
        project(k)
    acc_a, acc_b = acc

    out = g * acc_a[0:1, :] + (1.0 - g) * acc_b[0:1, :]
    o_ref[0] = out.astype(o_ref.dtype)


@jax.jit
def pallas_gated_mix__compressed_kv_cla__gqa_block_cached__decode_kernel(
    A_x: jax.Array,
    A_c_kv: jax.Array,
    A_w_q: jax.Array,
    A_w_uk: jax.Array,
    A_w_uv: jax.Array,
    A_w_o: jax.Array,
    B_x: jax.Array,
    B_k_cache: jax.Array,
    B_v_cache: jax.Array,
    B_wq: jax.Array,
    B_wo: jax.Array,
    gate_w: jax.Array,
):
    del B_x
    any_spec = pl.BlockSpec(memory_space=pl.ANY)
    return pl.pallas_call(
        _kernel,
        out_shape=jax.ShapeDtypeStruct((1, 1, M), A_x.dtype),
        in_specs=[any_spec] * 11,
        out_specs=pl.BlockSpec(memory_space=pltpu.VMEM),
        scratch_shapes=[
            pltpu.VMEM((1, 1, M), BF16),
            pltpu.VMEM((M,), BF16),
            pltpu.VMEM((SK, DC), BF16),
            pltpu.VMEM((M, H, D), BF16),
            pltpu.VMEM((DC, H, D), BF16),
            pltpu.VMEM((DC, H, D), BF16),
            pltpu.VMEM((H, D, M), BF16),
            pltpu.VMEM((H * SK, D), BF16),
            pltpu.VMEM((H * SK, D), BF16),
            pltpu.VMEM((M, H * D), BF16),
            pltpu.VMEM((H * D, M), BF16),
            pltpu.VMEM((M, 128), F32),
            pltpu.VMEM((8, H * D), F32),
            pltpu.VMEM((H, 8, D), F32),
            pltpu.VMEM((H, D), F32),
            pltpu.VMEM((H, DC), F32),
            pltpu.VMEM((H, SK), F32),
            pltpu.VMEM((DC // 128, H, 128), F32),
            pltpu.VMEM((H, D), F32),
            pltpu.VMEM((H, 8, D), F32),
            pltpu.SemaphoreType.DMA((RING,)),
            pltpu.SemaphoreType.DMA((RING,)),
        ],
        compiler_params=pltpu.CompilerParams(vmem_limit_bytes=112 * 1024 * 1024),
    )(A_x, A_c_kv, A_w_q, A_w_uk, A_w_uv, A_w_o,
      B_k_cache.reshape(H * SK, D), B_v_cache.reshape(H * SK, D),
      B_wq, B_wo, gate_w)
```

```python
import jax
import jax.numpy as jnp
import jax.experimental.pallas as pl
import jax.experimental.pallas.tpu as pltpu

F32 = jnp.float32
BF16 = jnp.bfloat16

M = 640
H = 32
D = 128
DC = 512
SK = 4096
SCALE = D ** -0.5
RING = 3

KV_PHASE = 64
WO_TILES = D * M // (8 * 128)
WOA_PHASE = 0
WOB_PHASE = 8


def _kernel(
    x_hbm, ckv_hbm, wqa_hbm, wuk_hbm, wuv_hbm, woa_hbm, k_hbm, v_hbm, wqb_hbm, wob_hbm, gate_hbm,
    o_ref,
    x_v, gate_v, ckv, wqa, wuk, wuv, woa, kb, vb, wqb, wob,
    xcol, qb_acc, q_scr, qa_scr, r_scr, s_scr, cc_scr, ctx_scr, o_scr,
    sem0, sem1,
):
    sems = (sem0, sem1)

    def start(src, dst, queue, sl):
        pltpu.make_async_copy(src, dst, sems[queue].at[sl]).start(priority=queue)

    def wait_all(dst, queue, sl):
        pltpu.make_async_copy(dst, dst, sems[queue].at[sl]).wait()

    def slot(s):
        return s % RING if isinstance(s, int) else jax.lax.rem(s, RING)

    def rounds(j0, j1, streams, fn):
        def body(j, c):
            for s in range(streams):
                fn(s, j)
            return c
        jax.lax.fori_loop(j0, j1, body, 0)

    def d_wqb(u, sl):
        r = pl.multiple_of((u // 8) * 8, 8)
        c = pl.multiple_of((u % 8) * 512, 128)
        start(wqb_hbm.at[pl.ds(r, 8), pl.ds(c, 2048)], wqb.at[pl.ds(r, 8), pl.ds(c, 2048)], 0, sl)

    def d_slab(src, dst, u, q, sl):
        start(src.at[pl.ds(u, 4)], dst.at[pl.ds(u, 4)], q, sl)

    def d_ckv(u, sl):
        r = pl.multiple_of(u * 8, 8)
        start(ckv_hbm.at[0, pl.ds(r, 32), :], ckv.at[pl.ds(r, 32), :], 1, sl)

    def d_kv(r, n, sl):
        start(k_hbm.at[pl.ds(r, n), :], kb.at[pl.ds(r, n), :], 0, sl)
        start(v_hbm.at[pl.ds(r, n), :], vb.at[pl.ds(r, n), :], 1, sl)

    def d_tiles(src, dst, ts, td, n, q, sl):
        start(src.at[pl.ds(ts, n)], dst.at[pl.ds(td, n)], q, sl)

    def wo_pieces(phase):
        cuts = [0] + [t for t in range(phase, WO_TILES, 16) if t > 0] + [WO_TILES]
        return [(a, b - a) for a, b in zip(cuts[:-1], cuts[1:])]

    def streams(u0, ns, parts, fns):
        def issue(part, sl):
            def f(s, j):
                for fn in fns:
                    fn(u0 + s * 64 + j * 4, sl)
            rounds(parts[part][0], parts[part][1], ns, f)
        return issue

    def win_q(r0, n):
        ns = n // 64
        parts = [(0, 8), (8, 16)] if ns <= 4 else [(0, 5), (5, 10), (10, 16)]
        issue = streams(r0, ns, parts, [d_wqb, lambda u, sl: d_slab(wqa_hbm, wqa, u, 1, sl)])

        def wait(sl):
            wait_all(wqb.at[pl.ds(r0, n), :], 0, sl)
            wait_all(wqa.at[pl.ds(r0, n)], 1, sl)
        return issue, len(parts), wait

    def win_uk(t):
        issue = streams(t * 256, 4, [(0, 8), (8, 16)],
                        [lambda u, sl: d_slab(wuk_hbm, wuk, u, 0, sl), d_ckv])

        def wait(sl):
            wait_all(wuk.at[pl.ds(t * 256, 256)], 0, sl)
            wait_all(ckv.at[pl.ds(t * 2048, 2048), :], 1, sl)
        return issue, 2, wait

    def win_uv():
        issue = streams(0, 4, [(0, 8), (8, 16)],
                        [lambda u, sl: d_slab(wuv_hbm, wuv, u, 0, sl),
                         lambda u, sl: d_slab(wuv_hbm, wuv, 256 + u, 1, sl)])

        def wait(sl):
            wait_all(wuv.at[pl.ds(0, 256)], 0, sl)
            wait_all(wuv.at[pl.ds(256, 256)], 1, sl)
        return issue, 2, wait

    def win_kv(w):
        r0 = KV_PHASE + 2 * w * SK

        def full(s, j, sl):
            d_kv(pl.multiple_of(r0 + (s * 16 + j) * 128, 16), 128, sl)

        def issue(part, sl, first=False, last=False):
            if part == 0:
                if first and KV_PHASE:
                    d_kv(0, KV_PHASE, sl)
                rounds(0, 8, 4, lambda s, j: full(s, j, sl))
            elif last and KV_PHASE:
                rounds(8, 15, 4, lambda s, j: full(s, j, sl))
                for s in range(4):
                    d_kv(pl.multiple_of(r0 + (s * 16 + 15) * 128, 16),
                         128 - KV_PHASE if s == 3 else 128, sl)
            else:
                rounds(8, 16, 4, lambda s, j: full(s, j, sl))

        def wait(sl, first=False, last=False):
            lo = 0 if first else r0
            n = 2 * SK + (KV_PHASE if first else 0) - (KV_PHASE if last else 0)
            lo = lo if first else pl.multiple_of(lo, 16)
            wait_all(kb.at[pl.ds(lo, n), :], 0, sl)
            wait_all(vb.at[pl.ds(lo, n), :], 1, sl)
        return issue, 2, wait

    wo_pos = [0, 0]

    def wo_window(parts):
        pa0, pb0 = wo_pos
        plan, heads_a, heads_b = [], [], []
        for part in parts:
            rs = []
            for ha, hb in part:
                rs.append(([(h, wo_pos[0] + n) for n, h in enumerate(ha)],
                           [(h, wo_pos[1] + n) for n, h in enumerate(hb)]))
                heads_a += rs[-1][0]
                heads_b += rs[-1][1]
                wo_pos[0] += len(ha)
                wo_pos[1] += len(hb)
            plan.append(rs)
        na, nb = wo_pos[0] - pa0, wo_pos[1] - pb0

        def issue(part, sl):
            pa, pb = wo_pieces(WOA_PHASE), wo_pieces(WOB_PHASE)
            for ra, rb in plan[part]:
                for j in range(max(len(pa), len(pb))):
                    for s in range(max(len(ra), len(rb))):
                        if s < len(ra) and j < len(pa):
                            d_tiles(woa_hbm, woa, ra[s][0] * WO_TILES + pa[j][0],
                                    ra[s][1] * WO_TILES + pa[j][0], pa[j][1], 0, sl)
                        if s < len(rb) and j < len(pb):
                            d_tiles(wob_hbm, wob, rb[s][0] * WO_TILES + pb[j][0],
                                    rb[s][1] * WO_TILES + pb[j][0], pb[j][1], 1, sl)

        def wait(sl):
            if na:
                wait_all(woa.at[pl.ds(pa0 * WO_TILES, na * WO_TILES)], 0, sl)
            if nb:
                wait_all(wob.at[pl.ds(pb0 * WO_TILES, nb * WO_TILES)], 1, sl)
        return issue, wait, heads_a, heads_b

    def rnd(base, j):
        hs = [base + 4 * s + j for s in range(4)]
        return hs, hs

    wo_windows = [
        wo_window([[rnd(0, 0), rnd(0, 1)], [rnd(0, 2), rnd(0, 3)]]),
        wo_window([[rnd(16, 0), rnd(16, 1)]]),
        wo_window([[rnd(16, 2)]]),
        wo_window([[([19], [19]), ([23], [23])]]),
        wo_window([[([27], [27]), ([31], [])]]),
        wo_window([[([], [31])]]),
    ]

    def stage_qb(r0, n, xb):
        part = jnp.dot(xb[:, r0:r0 + n], wqb[pl.ds(r0, n), :], preferred_element_type=F32)
        if r0 == 0:
            qb_acc[...] = part
        else:
            part = part + qb_acc[...]
            for h in range(H):
                q_scr[h] = part[:, h * D:(h + 1) * D]

    def stage_qa(r0, n):
        unroll = 16

        def body(i, acc):
            for u in range(unroll):
                m = r0 + i * unroll + u
                acc = acc + xcol[pl.ds(m, 1), :] * wqa[m].astype(F32)
            return acc
        acc = jax.lax.fori_loop(0, n // unroll, body, jnp.zeros((H, D), F32))
        if r0 == 0:
            qa_scr[...] = acc
        else:
            qa_scr[...] += acc

    def stage_qabs(j):
        q = qa_scr[...]
        lane = jax.lax.broadcasted_iota(jnp.int32, (H, 128), 1)
        unroll = 16

        def body(i, r):
            for u in range(unroll):
                cl = i * unroll + u
                s = jnp.sum(wuk[j * 128 + cl].astype(F32) * q, axis=-1, keepdims=True)
                r = jnp.where(lane == cl, s, r)
            return r
        r_scr[:, j * 128:(j + 1) * 128] = jax.lax.fori_loop(
            0, 128 // unroll, body, jnp.zeros((H, 128), F32))

    KC = 1024

    def stage_a_scores():
        r = r_scr[...].astype(BF16)
        for t in range(SK // KC):
            s = jax.lax.dot_general(r, ckv[pl.ds(t * KC, KC), :], (((1,), (1,)), ((), ())),
                                    preferred_element_type=F32)
            s_scr[:, t * KC:(t + 1) * KC] = s * SCALE

    def stage_a_softmax_pv():
        m = s_scr[:, 0:KC]
        for t in range(1, SK // KC):
            m = jnp.maximum(m, s_scr[:, t * KC:(t + 1) * KC])
        m = jnp.max(m, axis=-1, keepdims=True)
        l = jnp.zeros((H, 1), F32)
        acc = jnp.zeros((H, DC), F32)
        for t in range(SK // KC):
            p = jnp.exp(s_scr[:, t * KC:(t + 1) * KC] - m)
            l = l + jnp.sum(p, axis=-1, keepdims=True)
            acc = acc + jnp.dot(p.astype(BF16), ckv[pl.ds(t * KC, KC), :], preferred_element_type=F32)
        cc = acc / l
        for g in range(DC // 128):
            cc_scr[g] = cc[:, g * 128:(g + 1) * 128]

    def stage_ctx(g):
        cc = cc_scr[g]
        acc = ctx_scr[...]
        for cl in range(128):
            acc = acc + cc[:, cl:cl + 1] * wuv[g * 128 + cl].astype(F32)
        ctx_scr[...] = acc

    def stage_head(h):
        q = q_scr[h].astype(BF16)
        r = pl.multiple_of(h * SK, SK)
        s = jax.lax.dot_general(q, kb[pl.ds(r, SK), :], (((1,), (1,)), ((), ())),
                                preferred_element_type=F32) * SCALE
        m = jnp.max(s, axis=-1, keepdims=True)
        p = jnp.exp(s - m)
        l = jnp.sum(p, axis=-1, keepdims=True)
        o = jnp.dot(p.astype(BF16), vb[pl.ds(r, SK), :], preferred_element_type=F32)
        o_scr[h] = o / l

    windows = [win_q(0, 256), win_q(256, 384), win_uk(0), win_uk(1), win_uv()]
    n_static = len(windows)

    start(x_hbm, x_v, 0, 2)
    start(gate_hbm, gate_v, 1, 2)
    for part in range(windows[0][1]):
        windows[0][0](part, slot(0))
    wait_all(x_v, 0, 2)
    wait_all(gate_v, 1, 2)

    xf = x_v[0].astype(F32)
    xb = jnp.broadcast_to(xf, (8, M)).astype(BF16)
    xcol[...] = jnp.broadcast_to(xf, (128, M)).T
    gsum = jnp.sum(xf * gate_v[...].astype(F32).reshape(1, M), axis=-1, keepdims=True)
    g = jax.nn.sigmoid(gsum)
    ctx_scr[...] = jnp.zeros_like(ctx_scr)

    pieces = [
        [lambda: stage_qb(0, 256, xb), lambda: stage_qa(0, 256)],
        [lambda: stage_qb(256, 384, xb), lambda: stage_qa(256, 384)],
        [lambda: stage_qabs(0), lambda: stage_qabs(1)],
        [lambda: stage_qabs(2), lambda: stage_qabs(3)],
        [stage_a_scores, stage_a_softmax_pv],
    ]
    NW = H // 2
    kv0, kv1 = win_kv(0), win_kv(1)

    def issue(win, parts, n):
        for part in parts:
            win[0](part, slot(n))

    static_issue = [
        (lambda: issue(windows[1], (0, 1), 1), lambda: issue(windows[1], (2,), 1)),
        (lambda: issue(windows[2], (0, 1), 2), lambda: issue(windows[3], (0,), 3)),
        (lambda: issue(windows[3], (1,), 3), lambda: issue(windows[4], (0,), 4)),
        (lambda: issue(windows[4], (1,), 4), lambda: kv0[0](0, slot(5), first=True)),
        (lambda: issue(kv0, (1,), 5), lambda: issue(kv1, (0,), 6)),
    ]
    for n in range(n_static):
        static_issue[n][0]()
        windows[n][2](slot(n))
        pieces[n][0]()
        static_issue[n][1]()
        pieces[n][1]()

    n0 = n_static + NW

    def kv_body(w, c):
        n = n_static + w

        @pl.when(w < NW - 2)
        def _():
            win_kv(w + 1)[0](1, slot(n + 1))

        @pl.when(w == NW - 2)
        def _():
            win_kv(NW - 1)[0](1, slot(n_static + NW - 1), last=True)

        @pl.when(w == NW - 1)
        def _():
            wo_windows[0][0](1, slot(n0))

        @pl.when(w == 0)
        def _():
            win_kv(0)[2](slot(n_static), first=True)

        @pl.when(jnp.logical_and(w > 0, w < NW - 1))
        def _():
            win_kv(w)[2](slot(n))

        @pl.when(w == NW - 1)
        def _():
            win_kv(NW - 1)[2](slot(n_static + NW - 1), last=True)

        stage_head(2 * w)

        @pl.when(w < NW - 2)
        def _():
            win_kv(w + 2)[0](0, slot(n + 2))

        @pl.when(w == NW - 2)
        def _():
            wo_windows[0][0](0, slot(n0))

        @pl.when(w == NW - 1)
        def _():
            wo_windows[1][0](0, slot(n0 + 1))

        stage_head(2 * w + 1)

        @pl.when(w < DC // 128)
        def _():
            stage_ctx(w)
        return c
    jax.lax.fori_loop(0, NW, kv_body, 0)

    NJ = M // 128
    acc = [[jnp.zeros((8, 128), F32) for _ in range(NJ)] for _ in range(2)]

    def wo_tile(buf, p, j):
        return buf[pl.ds(p * WO_TILES + j, 16, stride=NJ)].reshape(128, 128)

    def project(k, lo=0, hi=None):
        _, _, heads_a, heads_b = wo_windows[k]
        for n in range(lo, max(len(heads_a), len(heads_b)) if hi is None else hi):
            if n < len(heads_a):
                h, p = heads_a[n]
                ctx_h = jnp.broadcast_to(ctx_scr[h:h + 1, :], (8, D)).astype(BF16)
                for j in range(NJ):
                    acc[0][j] = acc[0][j] + jnp.dot(ctx_h, wo_tile(woa, p, j),
                                                    preferred_element_type=F32)
            if n < len(heads_b):
                h, p = heads_b[n]
                o_h = o_scr[h].astype(BF16)
                for j in range(NJ):
                    acc[1][j] = acc[1][j] + jnp.dot(o_h, wo_tile(wob, p, j),
                                                    preferred_element_type=F32)

    def wo_issue(k):
        wo_windows[k][0](0, slot(n0 + k))

    def wo_wait(k):
        wo_windows[k][1](slot(n0 + k))

    wo_issue(2)
    wo_wait(0)
    project(0, 0, 8)
    wo_issue(3)
    project(0, 8, 16)
    wo_wait(1)
    wo_issue(4)
    project(1)
    wo_wait(2)
    wo_issue(5)
    project(2)
    for k in (3, 4, 5):
        wo_wait(k)
        project(k)
    acc_a, acc_b = (jnp.concatenate(a, axis=1) for a in acc)

    out = g * acc_a[0:1, :] + (1.0 - g) * acc_b[0:1, :]
    o_ref[0] = out.astype(o_ref.dtype)


def _tiles(w):
    r, c = w.shape
    return w.reshape(r // 8, 8, c // 128, 128).transpose(0, 2, 1, 3).reshape(r // 8 * (c // 128), 8, 128)


@jax.jit
def pallas_gated_mix__compressed_kv_cla__gqa_block_cached__decode_kernel(
    A_x: jax.Array,
    A_c_kv: jax.Array,
    A_w_q: jax.Array,
    A_w_uk: jax.Array,
    A_w_uv: jax.Array,
    A_w_o: jax.Array,
    B_x: jax.Array,
    B_k_cache: jax.Array,
    B_v_cache: jax.Array,
    B_wq: jax.Array,
    B_wo: jax.Array,
    gate_w: jax.Array,
):
    del B_x
    any_spec = pl.BlockSpec(memory_space=pl.ANY)
    return pl.pallas_call(
        _kernel,
        out_shape=jax.ShapeDtypeStruct((1, 1, M), A_x.dtype),
        in_specs=[any_spec] * 11,
        out_specs=pl.BlockSpec(memory_space=pltpu.VMEM),
        scratch_shapes=[
            pltpu.VMEM((1, 1, M), BF16),
            pltpu.VMEM((M,), BF16),
            pltpu.VMEM((SK, DC), BF16),
            pltpu.VMEM((M, H, D), BF16),
            pltpu.VMEM((DC, H, D), BF16),
            pltpu.VMEM((DC, H, D), BF16),
            pltpu.VMEM((H * WO_TILES, 8, 128), BF16),
            pltpu.VMEM((H * SK, D), BF16),
            pltpu.VMEM((H * SK, D), BF16),
            pltpu.VMEM((M, H * D), BF16),
            pltpu.VMEM((H * WO_TILES, 8, 128), BF16),
            pltpu.VMEM((M, 128), F32),
            pltpu.VMEM((8, H * D), F32),
            pltpu.VMEM((H, 8, D), F32),
            pltpu.VMEM((H, D), F32),
            pltpu.VMEM((H, DC), F32),
            pltpu.VMEM((H, SK), F32),
            pltpu.VMEM((DC // 128, H, 128), F32),
            pltpu.VMEM((H, D), F32),
            pltpu.VMEM((H, 8, D), F32),
            pltpu.SemaphoreType.DMA((RING,)),
            pltpu.SemaphoreType.DMA((RING,)),
        ],
        compiler_params=pltpu.CompilerParams(vmem_limit_bytes=112 * 1024 * 1024),
    )(A_x, A_c_kv, A_w_q, A_w_uk, A_w_uv, _tiles(A_w_o.reshape(H * D, M)),
      B_k_cache.reshape(H * SK, D), B_v_cache.reshape(H * SK, D),
      B_wq, _tiles(B_wo), gate_w)
```

```python
import jax
import jax.numpy as jnp
import jax.experimental.pallas as pl
import jax.experimental.pallas.tpu as pltpu

F32 = jnp.float32
BF16 = jnp.bfloat16

M = 640
H = 32
D = 128
DC = 512
SK = 4096
SCALE = D ** -0.5
RING = 3

KV_PHASE = 64
WO_TILES = D * M // (8 * 128)
WQ_TILES = M * H * D // (8 * 128)
WQB_PHASE = 8
WOA_PHASE = 0
WOB_PHASE = 8


def _kernel(
    x_hbm, ckv_hbm, wqa_hbm, wuk_hbm, wuv_hbm, woa_hbm, k_hbm, v_hbm, wqb_hbm, wob_hbm, gate_hbm,
    o_ref,
    x_v, gate_v, ckv, wqa, wuk, wuv, woa, kb, vb, wqb, wob,
    xcol, q_scr, qa_scr, r_scr, s_scr, cc_scr, ctx_scr, o_scr,
    sem0, sem1,
):
    sems = (sem0, sem1)

    def start(src, dst, queue, sl):
        pltpu.make_async_copy(src, dst, sems[queue].at[sl]).start(priority=queue)

    def wait_all(dst, queue, sl):
        pltpu.make_async_copy(dst, dst, sems[queue].at[sl]).wait()

    def slot(s):
        return s % RING if isinstance(s, int) else jax.lax.rem(s, RING)

    def rounds(j0, j1, streams, fn):
        def body(j, c):
            for s in range(streams):
                fn(s, j)
            return c
        jax.lax.fori_loop(j0, j1, body, 0)

    def d_slab(src, dst, u, q, sl):
        start(src.at[pl.ds(u, 4)], dst.at[pl.ds(u, 4)], q, sl)

    def d_ckv(u, sl):
        r = pl.multiple_of(u * 8, 8)
        start(ckv_hbm.at[0, pl.ds(r, 32), :], ckv.at[pl.ds(r, 32), :], 1, sl)

    def d_kv(r, n, sl):
        start(k_hbm.at[pl.ds(r, n), :], kb.at[pl.ds(r, n), :], 0, sl)
        start(v_hbm.at[pl.ds(r, n), :], vb.at[pl.ds(r, n), :], 1, sl)

    def d_tiles(src, dst, ts, td, n, q, sl):
        start(src.at[pl.ds(ts, n)], dst.at[pl.ds(td, n)], q, sl)

    def wo_pieces(phase):
        cuts = [0] + [t for t in range(phase, WO_TILES, 16) if t > 0] + [WO_TILES]
        return [(a, b - a) for a, b in zip(cuts[:-1], cuts[1:])]

    def streams(u0, ns, parts, fns):
        def issue(part, sl):
            def f(s, j):
                for fn in fns:
                    fn(u0 + s * 64 + j * 4, sl)
            rounds(parts[part][0], parts[part][1], ns, f)
        return issue

    def win_q(r0, n):
        ns = n // 64
        parts = [(0, 8), (8, 16)] if ns <= 4 else [(0, 5), (5, 10), (10, 16)]
        first, last = r0 == 0, r0 + n == M
        t0 = WQB_PHASE + r0 * 4

        def one(s, j, sl, short=False):
            u = s * 64 + j * 4
            d_tiles(wqb_hbm, wqb, t0 + u * 4, t0 + u * 4, 16 - WQB_PHASE if short else 16, 0, sl)
            d_slab(wqa_hbm, wqa, r0 + u, 1, sl)

        def issue(part, sl):
            lo, hi = parts[part]
            if first and part == 0 and WQB_PHASE:
                d_tiles(wqb_hbm, wqb, 0, 0, WQB_PHASE, 0, sl)
            tail = last and hi == 16 and WQB_PHASE > 0
            rounds(lo, hi - 1 if tail else hi, ns, lambda s, j: one(s, j, sl))
            if tail:
                for s in range(ns):
                    one(s, 15, sl, short=s == ns - 1)

        def wait(sl):
            lo = 0 if first else t0
            hi = WQ_TILES if last else t0 + n * 4
            wait_all(wqb.at[pl.ds(lo, hi - lo)], 0, sl)
            wait_all(wqa.at[pl.ds(r0, n)], 1, sl)
        return issue, len(parts), wait

    def win_uk(t):
        issue = streams(t * 256, 4, [(0, 8), (8, 16)],
                        [lambda u, sl: d_slab(wuk_hbm, wuk, u, 0, sl), d_ckv])

        def wait(sl):
            wait_all(wuk.at[pl.ds(t * 256, 256)], 0, sl)
            wait_all(ckv.at[pl.ds(t * 2048, 2048), :], 1, sl)
        return issue, 2, wait

    def win_uv():
        issue = streams(0, 4, [(0, 8), (8, 16)],
                        [lambda u, sl: d_slab(wuv_hbm, wuv, u, 0, sl),
                         lambda u, sl: d_slab(wuv_hbm, wuv, 256 + u, 1, sl)])

        def wait(sl):
            wait_all(wuv.at[pl.ds(0, 256)], 0, sl)
            wait_all(wuv.at[pl.ds(256, 256)], 1, sl)
        return issue, 2, wait

    def win_kv(w):
        r0 = KV_PHASE + 2 * w * SK

        def full(s, j, sl):
            d_kv(pl.multiple_of(r0 + (s * 16 + j) * 128, 16), 128, sl)

        def issue(part, sl, first=False, last=False):
            if part == 0:
                if first and KV_PHASE:
                    d_kv(0, KV_PHASE, sl)
                rounds(0, 8, 4, lambda s, j: full(s, j, sl))
            elif last and KV_PHASE:
                rounds(8, 15, 4, lambda s, j: full(s, j, sl))
                for s in range(4):
                    d_kv(pl.multiple_of(r0 + (s * 16 + 15) * 128, 16),
                         128 - KV_PHASE if s == 3 else 128, sl)
            else:
                rounds(8, 16, 4, lambda s, j: full(s, j, sl))

        def wait(sl, first=False, last=False):
            lo = 0 if first else r0
            n = 2 * SK + (KV_PHASE if first else 0) - (KV_PHASE if last else 0)
            lo = lo if first else pl.multiple_of(lo, 16)
            wait_all(kb.at[pl.ds(lo, n), :], 0, sl)
            wait_all(vb.at[pl.ds(lo, n), :], 1, sl)
        return issue, 2, wait

    wo_pos = [0, 0]

    def wo_window(parts):
        pa0, pb0 = wo_pos
        plan, heads_a, heads_b = [], [], []
        for part in parts:
            rs = []
            for ha, hb in part:
                rs.append(([(h, wo_pos[0] + n) for n, h in enumerate(ha)],
                           [(h, wo_pos[1] + n) for n, h in enumerate(hb)]))
                heads_a += rs[-1][0]
                heads_b += rs[-1][1]
                wo_pos[0] += len(ha)
                wo_pos[1] += len(hb)
            plan.append(rs)
        na, nb = wo_pos[0] - pa0, wo_pos[1] - pb0

        def issue(part, sl):
            pa, pb = wo_pieces(WOA_PHASE), wo_pieces(WOB_PHASE)
            for ra, rb in plan[part]:
                for j in range(max(len(pa), len(pb))):
                    for s in range(max(len(ra), len(rb))):
                        if s < len(ra) and j < len(pa):
                            d_tiles(woa_hbm, woa, ra[s][0] * WO_TILES + pa[j][0],
                                    ra[s][1] * WO_TILES + pa[j][0], pa[j][1], 0, sl)
                        if s < len(rb) and j < len(pb):
                            d_tiles(wob_hbm, wob, rb[s][0] * WO_TILES + pb[j][0],
                                    rb[s][1] * WO_TILES + pb[j][0], pb[j][1], 1, sl)

        def wait(sl):
            if na:
                wait_all(woa.at[pl.ds(pa0 * WO_TILES, na * WO_TILES)], 0, sl)
            if nb:
                wait_all(wob.at[pl.ds(pb0 * WO_TILES, nb * WO_TILES)], 1, sl)
        return issue, wait, heads_a, heads_b

    def rnd(base, j):
        hs = [base + 4 * s + j for s in range(4)]
        return hs, hs

    wo_windows = [
        wo_window([[rnd(0, 0), rnd(0, 1)], [rnd(0, 2), rnd(0, 3)]]),
        wo_window([[rnd(16, 0), rnd(16, 1)]]),
        wo_window([[rnd(16, 2)]]),
        wo_window([[([19], [19]), ([23], [23])]]),
        wo_window([[([27], [27]), ([31], [])]]),
        wo_window([[([], [31])]]),
    ]

    def stage_qb(r0, n, xb):
        for h in range(H):
            part = None
            for kb0 in range(r0, r0 + n, 128):
                w = wqb[pl.ds(kb0 * 4 + h, 16, stride=H)].reshape(128, 128)
                d = jnp.dot(xb[:, kb0:kb0 + 128], w, preferred_element_type=F32)
                part = d if part is None else part + d
            q_scr[h] = part if r0 == 0 else q_scr[h] + part

    def stage_qa(r0, n):
        unroll = 16

        def body(i, acc):
            for u in range(unroll):
                m = r0 + i * unroll + u
                acc = acc + xcol[pl.ds(m, 1), :] * wqa[m].astype(F32)
            return acc
        acc = jax.lax.fori_loop(0, n // unroll, body, jnp.zeros((H, D), F32))
        if r0 == 0:
            qa_scr[...] = acc
        else:
            qa_scr[...] += acc

    def stage_qabs(j):
        q = qa_scr[...]
        lane = jax.lax.broadcasted_iota(jnp.int32, (H, 128), 1)
        unroll = 16

        def body(i, r):
            for u in range(unroll):
                cl = i * unroll + u
                s = jnp.sum(wuk[j * 128 + cl].astype(F32) * q, axis=-1, keepdims=True)
                r = jnp.where(lane == cl, s, r)
            return r
        r_scr[:, j * 128:(j + 1) * 128] = jax.lax.fori_loop(
            0, 128 // unroll, body, jnp.zeros((H, 128), F32))

    KC = 1024

    def stage_a_scores():
        r = r_scr[...].astype(BF16)
        for t in range(SK // KC):
            s = jax.lax.dot_general(r, ckv[pl.ds(t * KC, KC), :], (((1,), (1,)), ((), ())),
                                    preferred_element_type=F32)
            s_scr[:, t * KC:(t + 1) * KC] = s * SCALE

    def stage_a_softmax_pv():
        m = s_scr[:, 0:KC]
        for t in range(1, SK // KC):
            m = jnp.maximum(m, s_scr[:, t * KC:(t + 1) * KC])
        m = jnp.max(m, axis=-1, keepdims=True)
        l = jnp.zeros((H, 1), F32)
        acc = jnp.zeros((H, DC), F32)
        for t in range(SK // KC):
            p = jnp.exp(s_scr[:, t * KC:(t + 1) * KC] - m)
            l = l + jnp.sum(p, axis=-1, keepdims=True)
            acc = acc + jnp.dot(p.astype(BF16), ckv[pl.ds(t * KC, KC), :], preferred_element_type=F32)
        cc = acc / l
        for g in range(DC // 128):
            cc_scr[g] = cc[:, g * 128:(g + 1) * 128]

    def stage_ctx(g):
        cc = cc_scr[g]
        acc = ctx_scr[...]
        for cl in range(128):
            acc = acc + cc[:, cl:cl + 1] * wuv[g * 128 + cl].astype(F32)
        ctx_scr[...] = acc

    def stage_head(h):
        q = q_scr[h].astype(BF16)
        r = pl.multiple_of(h * SK, SK)
        s = jax.lax.dot_general(q, kb[pl.ds(r, SK), :], (((1,), (1,)), ((), ())),
                                preferred_element_type=F32) * SCALE
        m = jnp.max(s, axis=-1, keepdims=True)
        p = jnp.exp(s - m)
        l = jnp.sum(p, axis=-1, keepdims=True)
        o = jnp.dot(p.astype(BF16), vb[pl.ds(r, SK), :], preferred_element_type=F32)
        o_scr[h] = o / l

    windows = [win_q(0, 256), win_q(256, 384), win_uk(0), win_uk(1), win_uv()]
    n_static = len(windows)

    start(x_hbm, x_v, 0, 2)
    start(gate_hbm, gate_v, 1, 2)
    for part in range(windows[0][1]):
        windows[0][0](part, slot(0))
    wait_all(x_v, 0, 2)
    wait_all(gate_v, 1, 2)

    xf = x_v[0].astype(F32)
    xb = jnp.broadcast_to(xf, (8, M)).astype(BF16)
    xcol[...] = jnp.broadcast_to(xf, (128, M)).T
    gsum = jnp.sum(xf * gate_v[...].astype(F32).reshape(1, M), axis=-1, keepdims=True)
    g = jax.nn.sigmoid(gsum)
    ctx_scr[...] = jnp.zeros_like(ctx_scr)

    pieces = [
        [lambda: stage_qb(0, 256, xb), lambda: stage_qa(0, 256)],
        [lambda: stage_qb(256, 384, xb), lambda: stage_qa(256, 384)],
        [lambda: stage_qabs(0), lambda: stage_qabs(1)],
        [lambda: stage_qabs(2), lambda: stage_qabs(3)],
        [stage_a_scores, stage_a_softmax_pv],
    ]
    NW = H // 2
    kv0, kv1 = win_kv(0), win_kv(1)

    def issue(win, parts, n):
        for part in parts:
            win[0](part, slot(n))

    static_issue = [
        (lambda: issue(windows[1], (0, 1), 1), lambda: issue(windows[1], (2,), 1)),
        (lambda: issue(windows[2], (0, 1), 2), lambda: issue(windows[3], (0,), 3)),
        (lambda: issue(windows[3], (1,), 3), lambda: issue(windows[4], (0,), 4)),
        (lambda: issue(windows[4], (1,), 4), lambda: kv0[0](0, slot(5), first=True)),
        (lambda: issue(kv0, (1,), 5), lambda: issue(kv1, (0,), 6)),
    ]
    for n in range(n_static):
        static_issue[n][0]()
        windows[n][2](slot(n))
        pieces[n][0]()
        static_issue[n][1]()
        pieces[n][1]()

    n0 = n_static + NW

    def kv_body(w, c):
        n = n_static + w

        @pl.when(w < NW - 2)
        def _():
            win_kv(w + 1)[0](1, slot(n + 1))

        @pl.when(w == NW - 2)
        def _():
            win_kv(NW - 1)[0](1, slot(n_static + NW - 1), last=True)

        @pl.when(w == NW - 1)
        def _():
            wo_windows[0][0](1, slot(n0))

        @pl.when(w == 0)
        def _():
            win_kv(0)[2](slot(n_static), first=True)

        @pl.when(jnp.logical_and(w > 0, w < NW - 1))
        def _():
            win_kv(w)[2](slot(n))

        @pl.when(w == NW - 1)
        def _():
            win_kv(NW - 1)[2](slot(n_static + NW - 1), last=True)

        stage_head(2 * w)

        @pl.when(w < NW - 2)
        def _():
            win_kv(w + 2)[0](0, slot(n + 2))

        @pl.when(w == NW - 2)
        def _():
            wo_windows[0][0](0, slot(n0))

        @pl.when(w == NW - 1)
        def _():
            wo_windows[1][0](0, slot(n0 + 1))

        stage_head(2 * w + 1)

        @pl.when(w < DC // 128)
        def _():
            stage_ctx(w)
        return c
    jax.lax.fori_loop(0, NW, kv_body, 0)

    NJ = M // 128
    acc = [[jnp.zeros((8, 128), F32) for _ in range(NJ)] for _ in range(2)]

    def wo_tile(buf, p, j):
        return buf[pl.ds(p * WO_TILES + j, 16, stride=NJ)].reshape(128, 128)

    def project(k, lo=0, hi=None):
        _, _, heads_a, heads_b = wo_windows[k]
        for n in range(lo, max(len(heads_a), len(heads_b)) if hi is None else hi):
            if n < len(heads_a):
                h, p = heads_a[n]
                ctx_h = jnp.broadcast_to(ctx_scr[h:h + 1, :], (8, D)).astype(BF16)
                for j in range(NJ):
                    acc[0][j] = acc[0][j] + jnp.dot(ctx_h, wo_tile(woa, p, j),
                                                    preferred_element_type=F32)
            if n < len(heads_b):
                h, p = heads_b[n]
                o_h = o_scr[h].astype(BF16)
                for j in range(NJ):
                    acc[1][j] = acc[1][j] + jnp.dot(o_h, wo_tile(wob, p, j),
                                                    preferred_element_type=F32)

    def wo_issue(k):
        wo_windows[k][0](0, slot(n0 + k))

    def wo_wait(k):
        wo_windows[k][1](slot(n0 + k))

    wo_issue(2)
    wo_wait(0)
    project(0, 0, 8)
    wo_issue(3)
    project(0, 8, 16)
    wo_wait(1)
    wo_issue(4)
    project(1)
    wo_wait(2)
    wo_issue(5)
    project(2)
    for k in (3, 4, 5):
        wo_wait(k)
        project(k)
    acc_a, acc_b = (jnp.concatenate(a, axis=1) for a in acc)

    out = g * acc_a[0:1, :] + (1.0 - g) * acc_b[0:1, :]
    o_ref[0] = out.astype(o_ref.dtype)


def _tiles(w):
    r, c = w.shape
    return w.reshape(r // 8, 8, c // 128, 128).transpose(0, 2, 1, 3).reshape(r // 8 * (c // 128), 8, 128)


@jax.jit
def pallas_gated_mix__compressed_kv_cla__gqa_block_cached__decode_kernel(
    A_x: jax.Array,
    A_c_kv: jax.Array,
    A_w_q: jax.Array,
    A_w_uk: jax.Array,
    A_w_uv: jax.Array,
    A_w_o: jax.Array,
    B_x: jax.Array,
    B_k_cache: jax.Array,
    B_v_cache: jax.Array,
    B_wq: jax.Array,
    B_wo: jax.Array,
    gate_w: jax.Array,
):
    del B_x
    any_spec = pl.BlockSpec(memory_space=pl.ANY)
    return pl.pallas_call(
        _kernel,
        out_shape=jax.ShapeDtypeStruct((1, 1, M), A_x.dtype),
        in_specs=[any_spec] * 11,
        out_specs=pl.BlockSpec(memory_space=pltpu.VMEM),
        scratch_shapes=[
            pltpu.VMEM((1, 1, M), BF16),
            pltpu.VMEM((M,), BF16),
            pltpu.VMEM((SK, DC), BF16),
            pltpu.VMEM((M, H, D), BF16),
            pltpu.VMEM((DC, H, D), BF16),
            pltpu.VMEM((DC, H, D), BF16),
            pltpu.VMEM((H * WO_TILES, 8, 128), BF16),
            pltpu.VMEM((H * SK, D), BF16),
            pltpu.VMEM((H * SK, D), BF16),
            pltpu.VMEM((WQ_TILES, 8, 128), BF16),
            pltpu.VMEM((H * WO_TILES, 8, 128), BF16),
            pltpu.VMEM((M, 128), F32),
            pltpu.VMEM((H, 8, D), F32),
            pltpu.VMEM((H, D), F32),
            pltpu.VMEM((H, DC), F32),
            pltpu.VMEM((H, SK), F32),
            pltpu.VMEM((DC // 128, H, 128), F32),
            pltpu.VMEM((H, D), F32),
            pltpu.VMEM((H, 8, D), F32),
            pltpu.SemaphoreType.DMA((RING,)),
            pltpu.SemaphoreType.DMA((RING,)),
        ],
        compiler_params=pltpu.CompilerParams(vmem_limit_bytes=112 * 1024 * 1024),
    )(A_x, A_c_kv, A_w_q, A_w_uk, A_w_uv, _tiles(A_w_o.reshape(H * D, M)),
      B_k_cache.reshape(H * SK, D), B_v_cache.reshape(H * SK, D),
      _tiles(B_wq), _tiles(B_wo), gate_w)
```

```python
import jax
import jax.numpy as jnp
import jax.experimental.pallas as pl
import jax.experimental.pallas.tpu as pltpu

F32 = jnp.float32
BF16 = jnp.bfloat16

M = 640
H = 32
D = 128
DC = 512
SK = 4096
SCALE = D ** -0.5
RING = 3

KV_PHASE = 64
WO_TILES = D * M // (8 * 128)
WQ_TILES = M * H * D // (8 * 128)
WQB_PHASE = 8
WOA_PHASE = 0
WOB_PHASE = 8


def _kernel(
    x_hbm, ckv_hbm, wqa_hbm, wuk_hbm, wuv_hbm, woa_hbm, k_hbm, v_hbm, wqb_hbm, wob_hbm, gate_hbm,
    o_ref,
    x_v, gate_v, ckv, wqa, wuk, wuv, woa, kb, vb, wqb, wob,
    xcol, q_scr, qa_scr, r_scr, s_scr, cc_scr, ctx_scr, o_scr,
    sem0, sem1,
):
    sems = (sem0, sem1)

    def start(src, dst, queue, sl):
        pltpu.make_async_copy(src, dst, sems[queue].at[sl]).start(priority=queue)

    def wait_all(dst, queue, sl):
        pltpu.make_async_copy(dst, dst, sems[queue].at[sl]).wait()

    def slot(s):
        return s % RING if isinstance(s, int) else jax.lax.rem(s, RING)

    def rounds(j0, j1, streams, fn):
        def body(j, c):
            for s in range(streams):
                fn(s, j)
            return c
        jax.lax.fori_loop(j0, j1, body, 0)

    def d_slab(src, dst, u, q, sl):
        start(src.at[pl.ds(u, 4)], dst.at[pl.ds(u, 4)], q, sl)

    def d_ckv(u, sl):
        r = pl.multiple_of(u * 8, 8)
        start(ckv_hbm.at[0, pl.ds(r, 32), :], ckv.at[pl.ds(r, 32), :], 1, sl)

    def d_kv(r, n, sl):
        start(k_hbm.at[pl.ds(r, n), :], kb.at[pl.ds(r, n), :], 0, sl)
        start(v_hbm.at[pl.ds(r, n), :], vb.at[pl.ds(r, n), :], 1, sl)

    def d_tiles(src, dst, ts, td, n, q, sl):
        start(src.at[pl.ds(ts, n)], dst.at[pl.ds(td, n)], q, sl)

    def wo_pieces(phase):
        cuts = [0] + [t for t in range(phase, WO_TILES, 16) if t > 0] + [WO_TILES]
        return [(a, b - a) for a, b in zip(cuts[:-1], cuts[1:])]

    def streams(u0, ns, parts, fns):
        def issue(part, sl):
            def f(s, j):
                for fn in fns:
                    fn(u0 + s * 64 + j * 4, sl)
            rounds(parts[part][0], parts[part][1], ns, f)
        return issue

    def win_q(r0, n):
        ns = n // 64
        parts = [(0, 8), (8, 16)] if ns <= 4 else [(0, 5), (5, 10), (10, 16)]
        first, last = r0 == 0, r0 + n == M
        t0 = WQB_PHASE + r0 * 4

        def one(s, j, sl, short=False):
            u = s * 64 + j * 4
            d_tiles(wqb_hbm, wqb, t0 + u * 4, t0 + u * 4, 16 - WQB_PHASE if short else 16, 0, sl)
            d_slab(wqa_hbm, wqa, r0 + u, 1, sl)

        def issue(part, sl):
            lo, hi = parts[part]
            if first and part == 0 and WQB_PHASE:
                d_tiles(wqb_hbm, wqb, 0, 0, WQB_PHASE, 0, sl)
            tail = last and hi == 16 and WQB_PHASE > 0
            rounds(lo, hi - 1 if tail else hi, ns, lambda s, j: one(s, j, sl))
            if tail:
                for s in range(ns):
                    one(s, 15, sl, short=s == ns - 1)

        def wait(sl):
            lo = 0 if first else t0
            hi = WQ_TILES if last else t0 + n * 4
            wait_all(wqb.at[pl.ds(lo, hi - lo)], 0, sl)
            wait_all(wqa.at[pl.ds(r0, n)], 1, sl)
        return issue, len(parts), wait

    def win_uk(t):
        issue = streams(t * 256, 4, [(0, 8), (8, 16)],
                        [lambda u, sl: d_slab(wuk_hbm, wuk, u, 0, sl), d_ckv])

        def wait(sl):
            wait_all(wuk.at[pl.ds(t * 256, 256)], 0, sl)
            wait_all(ckv.at[pl.ds(t * 2048, 2048), :], 1, sl)
        return issue, 2, wait

    def win_uv():
        issue = streams(0, 4, [(0, 8), (8, 16)],
                        [lambda u, sl: d_slab(wuv_hbm, wuv, u, 0, sl),
                         lambda u, sl: d_slab(wuv_hbm, wuv, 256 + u, 1, sl)])

        def wait(sl):
            wait_all(wuv.at[pl.ds(0, 256)], 0, sl)
            wait_all(wuv.at[pl.ds(256, 256)], 1, sl)
        return issue, 2, wait

    def win_kv(w):
        r0 = KV_PHASE + 2 * w * SK

        def full(s, j, sl):
            d_kv(pl.multiple_of(r0 + (s * 16 + j) * 128, 16), 128, sl)

        def issue(part, sl, first=False, last=False):
            if part == 0:
                if first and KV_PHASE:
                    d_kv(0, KV_PHASE, sl)
                rounds(0, 8, 4, lambda s, j: full(s, j, sl))
            elif last and KV_PHASE:
                rounds(8, 15, 4, lambda s, j: full(s, j, sl))
                for s in range(4):
                    d_kv(pl.multiple_of(r0 + (s * 16 + 15) * 128, 16),
                         128 - KV_PHASE if s == 3 else 128, sl)
            else:
                rounds(8, 16, 4, lambda s, j: full(s, j, sl))

        def wait(sl, first=False, last=False):
            lo = 0 if first else r0
            n = 2 * SK + (KV_PHASE if first else 0) - (KV_PHASE if last else 0)
            lo = lo if first else pl.multiple_of(lo, 16)
            wait_all(kb.at[pl.ds(lo, n), :], 0, sl)
            wait_all(vb.at[pl.ds(lo, n), :], 1, sl)
        return issue, 2, wait

    wo_pos = [0, 0]

    def wo_window(parts):
        pa0, pb0 = wo_pos
        plan, heads_a, heads_b = [], [], []
        for part in parts:
            rs = []
            for ha, hb in part:
                rs.append(([(h, wo_pos[0] + n) for n, h in enumerate(ha)],
                           [(h, wo_pos[1] + n) for n, h in enumerate(hb)]))
                heads_a += rs[-1][0]
                heads_b += rs[-1][1]
                wo_pos[0] += len(ha)
                wo_pos[1] += len(hb)
            plan.append(rs)
        na, nb = wo_pos[0] - pa0, wo_pos[1] - pb0

        def issue(part, sl):
            pa, pb = wo_pieces(WOA_PHASE), wo_pieces(WOB_PHASE)
            for ra, rb in plan[part]:
                for j in range(max(len(pa), len(pb))):
                    for s in range(max(len(ra), len(rb))):
                        if s < len(ra) and j < len(pa):
                            d_tiles(woa_hbm, woa, ra[s][0] * WO_TILES + pa[j][0],
                                    ra[s][1] * WO_TILES + pa[j][0], pa[j][1], 0, sl)
                        if s < len(rb) and j < len(pb):
                            d_tiles(wob_hbm, wob, rb[s][0] * WO_TILES + pb[j][0],
                                    rb[s][1] * WO_TILES + pb[j][0], pb[j][1], 1, sl)

        def wait(sl):
            if na:
                wait_all(woa.at[pl.ds(pa0 * WO_TILES, na * WO_TILES)], 0, sl)
            if nb:
                wait_all(wob.at[pl.ds(pb0 * WO_TILES, nb * WO_TILES)], 1, sl)
        return issue, wait, heads_a, heads_b

    def rnd(base, j):
        hs = [base + 4 * s + j for s in range(4)]
        return hs, hs

    wo_windows = [
        wo_window([[rnd(0, 0), rnd(0, 1)], [rnd(0, 2), rnd(0, 3)]]),
        wo_window([[rnd(16, 0), rnd(16, 1)]]),
        wo_window([[rnd(16, 2)]]),
        wo_window([[([19], [19]), ([23], [23])]]),
        wo_window([[([27], [27]), ([31], [])]]),
        wo_window([[([], [31])]]),
    ]

    def tile_block(buf, t0, step):
        return jnp.concatenate([buf[t0 + a * step] for a in range(16)], axis=0)

    def stage_qb(r0, n, xb):
        for h in range(H):
            part = None
            for kb0 in range(r0, r0 + n, 128):
                w = tile_block(wqb, kb0 * 4 + h, H)
                d = jnp.dot(xb[:, kb0:kb0 + 128], w, preferred_element_type=F32)
                part = d if part is None else part + d
            q_scr[h] = part if r0 == 0 else q_scr[h] + part

    def stage_qa(r0, n):
        unroll = 16

        def body(i, acc):
            for u in range(unroll):
                m = r0 + i * unroll + u
                acc = acc + xcol[pl.ds(m, 1), :] * wqa[m].astype(F32)
            return acc
        acc = jax.lax.fori_loop(0, n // unroll, body, jnp.zeros((H, D), F32))
        if r0 == 0:
            qa_scr[...] = acc
        else:
            qa_scr[...] += acc

    def stage_qabs(j):
        q = qa_scr[...]
        lane = jax.lax.broadcasted_iota(jnp.int32, (H, 128), 1)
        unroll = 16

        def body(i, r):
            for u in range(unroll):
                cl = i * unroll + u
                s = jnp.sum(wuk[j * 128 + cl].astype(F32) * q, axis=-1, keepdims=True)
                r = jnp.where(lane == cl, s, r)
            return r
        r_scr[:, j * 128:(j + 1) * 128] = jax.lax.fori_loop(
            0, 128 // unroll, body, jnp.zeros((H, 128), F32))

    KC = 1024

    def stage_a_scores():
        r = r_scr[...].astype(BF16)
        for t in range(SK // KC):
            s = jax.lax.dot_general(r, ckv[pl.ds(t * KC, KC), :], (((1,), (1,)), ((), ())),
                                    preferred_element_type=F32)
            s_scr[:, t * KC:(t + 1) * KC] = s * SCALE

    def stage_a_softmax_pv():
        m = s_scr[:, 0:KC]
        for t in range(1, SK // KC):
            m = jnp.maximum(m, s_scr[:, t * KC:(t + 1) * KC])
        m = jnp.max(m, axis=-1, keepdims=True)
        l = jnp.zeros((H, 1), F32)
        acc = jnp.zeros((H, DC), F32)
        for t in range(SK // KC):
            p = jnp.exp(s_scr[:, t * KC:(t + 1) * KC] - m)
            l = l + jnp.sum(p, axis=-1, keepdims=True)
            acc = acc + jnp.dot(p.astype(BF16), ckv[pl.ds(t * KC, KC), :], preferred_element_type=F32)
        cc = acc / l
        for g in range(DC // 128):
            cc_scr[g] = cc[:, g * 128:(g + 1) * 128]

    def stage_ctx(g):
        cc = cc_scr[g]
        acc = ctx_scr[...]
        for cl in range(128):
            acc = acc + cc[:, cl:cl + 1] * wuv[g * 128 + cl].astype(F32)
        ctx_scr[...] = acc

    def stage_head(h):
        q = q_scr[h].astype(BF16)
        r = pl.multiple_of(h * SK, SK)
        s = jax.lax.dot_general(q, kb[pl.ds(r, SK), :], (((1,), (1,)), ((), ())),
                                preferred_element_type=F32) * SCALE
        m = jnp.max(s, axis=-1, keepdims=True)
        p = jnp.exp(s - m)
        l = jnp.sum(p, axis=-1, keepdims=True)
        o = jnp.dot(p.astype(BF16), vb[pl.ds(r, SK), :], preferred_element_type=F32)
        o_scr[h] = o / l

    windows = [win_q(0, 256), win_q(256, 384), win_uk(0), win_uk(1), win_uv()]
    n_static = len(windows)

    start(x_hbm, x_v, 0, 2)
    start(gate_hbm, gate_v, 1, 2)
    for part in range(windows[0][1]):
        windows[0][0](part, slot(0))
    wait_all(x_v, 0, 2)
    wait_all(gate_v, 1, 2)

    xf = x_v[0].astype(F32)
    xb = jnp.broadcast_to(xf, (8, M)).astype(BF16)
    xcol[...] = jnp.broadcast_to(xf, (128, M)).T
    gsum = jnp.sum(xf * gate_v[...].astype(F32).reshape(1, M), axis=-1, keepdims=True)
    g = jax.nn.sigmoid(gsum)
    ctx_scr[...] = jnp.zeros_like(ctx_scr)

    pieces = [
        [lambda: stage_qb(0, 256, xb), lambda: stage_qa(0, 256)],
        [lambda: stage_qb(256, 384, xb), lambda: stage_qa(256, 384)],
        [lambda: stage_qabs(0), lambda: stage_qabs(1)],
        [lambda: stage_qabs(2), lambda: stage_qabs(3)],
        [stage_a_scores, stage_a_softmax_pv],
    ]
    NW = H // 2
    kv0, kv1 = win_kv(0), win_kv(1)

    def issue(win, parts, n):
        for part in parts:
            win[0](part, slot(n))

    static_issue = [
        (lambda: issue(windows[1], (0, 1), 1), lambda: issue(windows[1], (2,), 1)),
        (lambda: issue(windows[2], (0, 1), 2), lambda: issue(windows[3], (0,), 3)),
        (lambda: issue(windows[3], (1,), 3), lambda: issue(windows[4], (0,), 4)),
        (lambda: issue(windows[4], (1,), 4), lambda: kv0[0](0, slot(5), first=True)),
        (lambda: issue(kv0, (1,), 5), lambda: issue(kv1, (0,), 6)),
    ]
    for n in range(n_static):
        static_issue[n][0]()
        windows[n][2](slot(n))
        pieces[n][0]()
        static_issue[n][1]()
        pieces[n][1]()

    n0 = n_static + NW

    def kv_body(w, c):
        n = n_static + w

        @pl.when(w < NW - 2)
        def _():
            win_kv(w + 1)[0](1, slot(n + 1))

        @pl.when(w == NW - 2)
        def _():
            win_kv(NW - 1)[0](1, slot(n_static + NW - 1), last=True)

        @pl.when(w == NW - 1)
        def _():
            wo_windows[0][0](1, slot(n0))

        @pl.when(w == 0)
        def _():
            win_kv(0)[2](slot(n_static), first=True)

        @pl.when(jnp.logical_and(w > 0, w < NW - 1))
        def _():
            win_kv(w)[2](slot(n))

        @pl.when(w == NW - 1)
        def _():
            win_kv(NW - 1)[2](slot(n_static + NW - 1), last=True)

        stage_head(2 * w)

        @pl.when(w < NW - 2)
        def _():
            win_kv(w + 2)[0](0, slot(n + 2))

        @pl.when(w == NW - 2)
        def _():
            wo_windows[0][0](0, slot(n0))

        @pl.when(w == NW - 1)
        def _():
            wo_windows[1][0](0, slot(n0 + 1))

        stage_head(2 * w + 1)

        @pl.when(w < DC // 128)
        def _():
            stage_ctx(w)
        return c
    jax.lax.fori_loop(0, NW, kv_body, 0)

    NJ = M // 128
    acc = [[jnp.zeros((8, 128), F32) for _ in range(NJ)] for _ in range(2)]

    def wo_tile(buf, p, j):
        return tile_block(buf, p * WO_TILES + j, NJ)

    def project(k, lo=0, hi=None):
        _, _, heads_a, heads_b = wo_windows[k]
        for n in range(lo, max(len(heads_a), len(heads_b)) if hi is None else hi):
            if n < len(heads_a):
                h, p = heads_a[n]
                ctx_h = jnp.broadcast_to(ctx_scr[h:h + 1, :], (8, D)).astype(BF16)
                for j in range(NJ):
                    acc[0][j] = acc[0][j] + jnp.dot(ctx_h, wo_tile(woa, p, j),
                                                    preferred_element_type=F32)
            if n < len(heads_b):
                h, p = heads_b[n]
                o_h = o_scr[h].astype(BF16)
                for j in range(NJ):
                    acc[1][j] = acc[1][j] + jnp.dot(o_h, wo_tile(wob, p, j),
                                                    preferred_element_type=F32)

    def wo_issue(k):
        wo_windows[k][0](0, slot(n0 + k))

    def wo_wait(k):
        wo_windows[k][1](slot(n0 + k))

    wo_issue(2)
    wo_wait(0)
    project(0, 0, 8)
    wo_issue(3)
    project(0, 8, 16)
    wo_wait(1)
    wo_issue(4)
    project(1)
    wo_wait(2)
    wo_issue(5)
    project(2)
    for k in (3, 4, 5):
        wo_wait(k)
        project(k)
    acc_a, acc_b = (jnp.concatenate(a, axis=1) for a in acc)

    out = g * acc_a[0:1, :] + (1.0 - g) * acc_b[0:1, :]
    o_ref[0] = out.astype(o_ref.dtype)


def _tiles(w):
    r, c = w.shape
    return w.reshape(r // 8, 8, c // 128, 128).transpose(0, 2, 1, 3).reshape(r // 8 * (c // 128), 8, 128)


@jax.jit
def pallas_gated_mix__compressed_kv_cla__gqa_block_cached__decode_kernel(
    A_x: jax.Array,
    A_c_kv: jax.Array,
    A_w_q: jax.Array,
    A_w_uk: jax.Array,
    A_w_uv: jax.Array,
    A_w_o: jax.Array,
    B_x: jax.Array,
    B_k_cache: jax.Array,
    B_v_cache: jax.Array,
    B_wq: jax.Array,
    B_wo: jax.Array,
    gate_w: jax.Array,
):
    del B_x
    any_spec = pl.BlockSpec(memory_space=pl.ANY)
    return pl.pallas_call(
        _kernel,
        out_shape=jax.ShapeDtypeStruct((1, 1, M), A_x.dtype),
        in_specs=[any_spec] * 11,
        out_specs=pl.BlockSpec(memory_space=pltpu.VMEM),
        scratch_shapes=[
            pltpu.VMEM((1, 1, M), BF16),
            pltpu.VMEM((M,), BF16),
            pltpu.VMEM((SK, DC), BF16),
            pltpu.VMEM((M, H, D), BF16),
            pltpu.VMEM((DC, H, D), BF16),
            pltpu.VMEM((DC, H, D), BF16),
            pltpu.VMEM((H * WO_TILES, 8, 128), BF16),
            pltpu.VMEM((H * SK, D), BF16),
            pltpu.VMEM((H * SK, D), BF16),
            pltpu.VMEM((WQ_TILES, 8, 128), BF16),
            pltpu.VMEM((H * WO_TILES, 8, 128), BF16),
            pltpu.VMEM((M, 128), F32),
            pltpu.VMEM((H, 8, D), F32),
            pltpu.VMEM((H, D), F32),
            pltpu.VMEM((H, DC), F32),
            pltpu.VMEM((H, SK), F32),
            pltpu.VMEM((DC // 128, H, 128), F32),
            pltpu.VMEM((H, D), F32),
            pltpu.VMEM((H, 8, D), F32),
            pltpu.SemaphoreType.DMA((RING,)),
            pltpu.SemaphoreType.DMA((RING,)),
        ],
        compiler_params=pltpu.CompilerParams(vmem_limit_bytes=112 * 1024 * 1024),
    )(A_x, A_c_kv, A_w_q, A_w_uk, A_w_uv, _tiles(A_w_o.reshape(H * D, M)),
      B_k_cache.reshape(H * SK, D), B_v_cache.reshape(H * SK, D),
      _tiles(B_wq), _tiles(B_wo), gate_w)
```

```python
import jax
import jax.numpy as jnp
import jax.experimental.pallas as pl
import jax.experimental.pallas.tpu as pltpu

F32 = jnp.float32
BF16 = jnp.bfloat16

M = 640
H = 32
D = 128
DC = 512
SK = 4096
SCALE = D ** -0.5
RING = 3

WO_TILES = D * M // (8 * 128)
WQ_TILES = M * H * D // (8 * 128)

KV_PHASE = 64
WQB_PHASE = 8
WOA_PHASE = 0
WOB_PHASE = 8


def _kernel(
    x_hbm, ckv_hbm, wqa_hbm, wuk_hbm, wuv_hbm, woa_hbm, k_hbm, v_hbm, wqb_hbm, wob_hbm, gate_hbm,
    o_ref,
    x_v, gate_v, ckv, wqa, wuk, wuv, woa, kb, vb, wqb, wob,
    xcol, q_scr, qa_scr, r_scr, s_scr, cc_scr, ctx_scr, o_scr,
    sem0, sem1,
):
    sems = (sem0, sem1)

    def start(src, dst, queue, sl):
        pltpu.make_async_copy(src, dst, sems[queue].at[sl]).start(priority=queue)

    def wait_all(dst, queue, sl):
        pltpu.make_async_copy(dst, dst, sems[queue].at[sl]).wait()

    def slot(s):
        return s % RING if isinstance(s, int) else jax.lax.rem(s, RING)

    def rounds(j0, j1, streams, fn):
        def body(j, c):
            for s in range(streams):
                fn(s, j)
            return c
        jax.lax.fori_loop(j0, j1, body, 0)

    def d_slab(src, dst, u, q, sl):
        start(src.at[pl.ds(u, 4)], dst.at[pl.ds(u, 4)], q, sl)

    def d_ckv(u, sl):
        r = pl.multiple_of(u * 8, 8)
        start(ckv_hbm.at[0, pl.ds(r, 32), :], ckv.at[pl.ds(r, 32), :], 1, sl)

    def d_kv(r, n, sl):
        start(k_hbm.at[pl.ds(r, n), :], kb.at[pl.ds(r, n), :], 0, sl)
        start(v_hbm.at[pl.ds(r, n), :], vb.at[pl.ds(r, n), :], 1, sl)

    def d_tiles(src, dst, ts, td, n, q, sl):
        start(src.at[pl.ds(ts, n)], dst.at[pl.ds(td, n)], q, sl)

    def wo_pieces(phase):
        cuts = [0] + [t for t in range(phase, WO_TILES, 16) if t > 0] + [WO_TILES]
        return [(a, b - a) for a, b in zip(cuts[:-1], cuts[1:])]

    def streams(u0, ns, parts, fns):
        def issue(part, sl):
            def f(s, j):
                for fn in fns:
                    fn(u0 + s * 64 + j * 4, sl)
            rounds(parts[part][0], parts[part][1], ns, f)
        return issue

    def win_q(r0, n):
        ns = n // 64
        parts = [(0, 8), (8, 16)] if ns <= 4 else [(0, 5), (5, 10), (10, 16)]
        first, last = r0 == 0, r0 + n == M
        t0 = WQB_PHASE + r0 * 4

        def one(s, j, sl, short=False):
            u = s * 64 + j * 4
            d_tiles(wqb_hbm, wqb, t0 + u * 4, t0 + u * 4, 16 - WQB_PHASE if short else 16, 0, sl)
            d_slab(wqa_hbm, wqa, r0 + u, 1, sl)

        def issue(part, sl):
            lo, hi = parts[part]
            if first and part == 0 and WQB_PHASE:
                d_tiles(wqb_hbm, wqb, 0, 0, WQB_PHASE, 0, sl)
            tail = last and hi == 16 and WQB_PHASE > 0
            rounds(lo, hi - 1 if tail else hi, ns, lambda s, j: one(s, j, sl))
            if tail:
                for s in range(ns):
                    one(s, 15, sl, short=s == ns - 1)

        def wait(sl):
            lo = 0 if first else t0
            hi = WQ_TILES if last else t0 + n * 4
            wait_all(wqb.at[pl.ds(lo, hi - lo)], 0, sl)
            wait_all(wqa.at[pl.ds(r0, n)], 1, sl)
        return issue, len(parts), wait

    def win_uk(t):
        issue = streams(t * 256, 4, [(0, 8), (8, 16)],
                        [lambda u, sl: d_slab(wuk_hbm, wuk, u, 0, sl), d_ckv])

        def wait(sl):
            wait_all(wuk.at[pl.ds(t * 256, 256)], 0, sl)
            wait_all(ckv.at[pl.ds(t * 2048, 2048), :], 1, sl)
        return issue, 2, wait

    def win_uv():
        issue = streams(0, 4, [(0, 8), (8, 16)],
                        [lambda u, sl: d_slab(wuv_hbm, wuv, u, 0, sl),
                         lambda u, sl: d_slab(wuv_hbm, wuv, 256 + u, 1, sl)])

        def wait(sl):
            wait_all(wuv.at[pl.ds(0, 256)], 0, sl)
            wait_all(wuv.at[pl.ds(256, 256)], 1, sl)
        return issue, 2, wait

    def win_kv(w):
        r0 = KV_PHASE + 2 * w * SK

        def full(s, j, sl):
            d_kv(pl.multiple_of(r0 + (s * 16 + j) * 128, 16), 128, sl)

        def issue(part, sl, first=False, last=False):
            if part == 0:
                if first and KV_PHASE:
                    d_kv(0, KV_PHASE, sl)
                rounds(0, 8, 4, lambda s, j: full(s, j, sl))
            elif last and KV_PHASE:
                rounds(8, 15, 4, lambda s, j: full(s, j, sl))
                for s in range(4):
                    d_kv(pl.multiple_of(r0 + (s * 16 + 15) * 128, 16),
                         128 - KV_PHASE if s == 3 else 128, sl)
            else:
                rounds(8, 16, 4, lambda s, j: full(s, j, sl))

        def wait(sl, first=False, last=False):
            lo = 0 if first else r0
            n = 2 * SK + (KV_PHASE if first else 0) - (KV_PHASE if last else 0)
            lo = lo if first else pl.multiple_of(lo, 16)
            wait_all(kb.at[pl.ds(lo, n), :], 0, sl)
            wait_all(vb.at[pl.ds(lo, n), :], 1, sl)
        return issue, 2, wait

    wo_pos = [0, 0]

    def wo_window(parts):
        pa0, pb0 = wo_pos
        plan, heads_a, heads_b = [], [], []
        for part in parts:
            rs = []
            for ha, hb in part:
                rs.append(([(h, wo_pos[0] + n) for n, h in enumerate(ha)],
                           [(h, wo_pos[1] + n) for n, h in enumerate(hb)]))
                heads_a += rs[-1][0]
                heads_b += rs[-1][1]
                wo_pos[0] += len(ha)
                wo_pos[1] += len(hb)
            plan.append(rs)
        na, nb = wo_pos[0] - pa0, wo_pos[1] - pb0

        def issue(part, sl):
            pa, pb = wo_pieces(WOA_PHASE), wo_pieces(WOB_PHASE)
            for ra, rb in plan[part]:
                for j in range(max(len(pa), len(pb))):
                    for s in range(max(len(ra), len(rb))):
                        if s < len(ra) and j < len(pa):
                            d_tiles(woa_hbm, woa, ra[s][0] * WO_TILES + pa[j][0],
                                    ra[s][1] * WO_TILES + pa[j][0], pa[j][1], 0, sl)
                        if s < len(rb) and j < len(pb):
                            d_tiles(wob_hbm, wob, rb[s][0] * WO_TILES + pb[j][0],
                                    rb[s][1] * WO_TILES + pb[j][0], pb[j][1], 1, sl)

        def wait(sl):
            if na:
                wait_all(woa.at[pl.ds(pa0 * WO_TILES, na * WO_TILES)], 0, sl)
            if nb:
                wait_all(wob.at[pl.ds(pb0 * WO_TILES, nb * WO_TILES)], 1, sl)
        return issue, wait, heads_a, heads_b

    def rnd(base, j):
        hs = [base + 4 * s + j for s in range(4)]
        return hs, hs

    wo_windows = [
        wo_window([[rnd(0, 0), rnd(0, 1)], [rnd(0, 2), rnd(0, 3)]]),
        wo_window([[rnd(16, 0), rnd(16, 1)]]),
        wo_window([[rnd(16, 2)]]),
        wo_window([[([19], [19]), ([23], [23])]]),
        wo_window([[([27], [27]), ([31], [])]]),
        wo_window([[([], [31])]]),
    ]

    def stage_qb(r0, n, xb):
        parts = [None] * H
        for kb0 in range(r0, r0 + n, 128):
            w = wqb[pl.ds(kb0 * 4, 16 * H)].reshape(16, H, 8, 128)
            for h in range(H):
                d = jnp.dot(xb[:, kb0:kb0 + 128], w[:, h].reshape(128, 128),
                            preferred_element_type=F32)
                parts[h] = d if parts[h] is None else parts[h] + d
        for h in range(H):
            q_scr[h] = parts[h] if r0 == 0 else q_scr[h] + parts[h]

    def stage_qa(r0, n):
        unroll = 16

        def body(i, acc):
            for u in range(unroll):
                m = r0 + i * unroll + u
                acc = acc + xcol[pl.ds(m, 1), :] * wqa[m].astype(F32)
            return acc
        acc = jax.lax.fori_loop(0, n // unroll, body, jnp.zeros((H, D), F32))
        if r0 == 0:
            qa_scr[...] = acc
        else:
            qa_scr[...] += acc

    def stage_qabs(j):
        q = qa_scr[...]
        lane = jax.lax.broadcasted_iota(jnp.int32, (H, 128), 1)
        unroll = 16

        def body(i, r):
            for u in range(unroll):
                cl = i * unroll + u
                s = jnp.sum(wuk[j * 128 + cl].astype(F32) * q, axis=-1, keepdims=True)
                r = jnp.where(lane == cl, s, r)
            return r
        r_scr[:, j * 128:(j + 1) * 128] = jax.lax.fori_loop(
            0, 128 // unroll, body, jnp.zeros((H, 128), F32))

    KC = 1024

    def stage_a_scores():
        r = r_scr[...].astype(BF16)
        for t in range(SK // KC):
            s = jax.lax.dot_general(r, ckv[pl.ds(t * KC, KC), :], (((1,), (1,)), ((), ())),
                                    preferred_element_type=F32)
            s_scr[:, t * KC:(t + 1) * KC] = s * SCALE

    def stage_a_softmax_pv():
        m = s_scr[:, 0:KC]
        for t in range(1, SK // KC):
            m = jnp.maximum(m, s_scr[:, t * KC:(t + 1) * KC])
        m = jnp.max(m, axis=-1, keepdims=True)
        l = jnp.zeros((H, 1), F32)
        acc = jnp.zeros((H, DC), F32)
        for t in range(SK // KC):
            p = jnp.exp(s_scr[:, t * KC:(t + 1) * KC] - m)
            l = l + jnp.sum(p, axis=-1, keepdims=True)
            acc = acc + jnp.dot(p.astype(BF16), ckv[pl.ds(t * KC, KC), :], preferred_element_type=F32)
        cc = acc / l
        for g in range(DC // 128):
            cc_scr[g] = cc[:, g * 128:(g + 1) * 128]

    def stage_ctx(g):
        cc = cc_scr[g]
        acc = ctx_scr[...]
        for cl in range(128):
            acc = acc + cc[:, cl:cl + 1] * wuv[g * 128 + cl].astype(F32)
        ctx_scr[...] = acc

    def stage_head(h):
        q = q_scr[h].astype(BF16)
        r = pl.multiple_of(h * SK, SK)
        s = jax.lax.dot_general(q, kb[pl.ds(r, SK), :], (((1,), (1,)), ((), ())),
                                preferred_element_type=F32) * SCALE
        m = jnp.max(s, axis=-1, keepdims=True)
        p = jnp.exp(s - m)
        l = jnp.sum(p, axis=-1, keepdims=True)
        o = jnp.dot(p.astype(BF16), vb[pl.ds(r, SK), :], preferred_element_type=F32)
        o_scr[h] = o / l

    windows = [win_q(0, 256), win_q(256, 384), win_uk(0), win_uk(1), win_uv()]
    n_static = len(windows)

    start(x_hbm, x_v, 0, 2)
    start(gate_hbm, gate_v, 1, 2)
    for part in range(windows[0][1]):
        windows[0][0](part, slot(0))
    wait_all(x_v, 0, 2)
    wait_all(gate_v, 1, 2)

    xf = x_v[0].astype(F32)
    xb = jnp.broadcast_to(xf, (8, M)).astype(BF16)
    xcol[...] = jnp.broadcast_to(xf, (128, M)).T
    gsum = jnp.sum(xf * gate_v[...].astype(F32).reshape(1, M), axis=-1, keepdims=True)
    g = jax.nn.sigmoid(gsum)
    ctx_scr[...] = jnp.zeros_like(ctx_scr)

    pieces = [
        [lambda: stage_qb(0, 256, xb), lambda: stage_qa(0, 256)],
        [lambda: stage_qb(256, 384, xb), lambda: stage_qa(256, 384)],
        [lambda: stage_qabs(0), lambda: stage_qabs(1)],
        [lambda: stage_qabs(2), lambda: stage_qabs(3)],
        [stage_a_scores, stage_a_softmax_pv],
    ]
    NW = H // 2
    kv0, kv1 = win_kv(0), win_kv(1)

    def issue(win, parts, n):
        for part in parts:
            win[0](part, slot(n))

    static_issue = [
        (lambda: issue(windows[1], (0, 1), 1), lambda: issue(windows[1], (2,), 1)),
        (lambda: issue(windows[2], (0, 1), 2), lambda: issue(windows[3], (0,), 3)),
        (lambda: issue(windows[3], (1,), 3), lambda: issue(windows[4], (0,), 4)),
        (lambda: issue(windows[4], (1,), 4), lambda: kv0[0](0, slot(5), first=True)),
        (lambda: issue(kv0, (1,), 5), lambda: issue(kv1, (0,), 6)),
    ]
    for n in range(n_static):
        static_issue[n][0]()
        windows[n][2](slot(n))
        pieces[n][0]()
        static_issue[n][1]()
        pieces[n][1]()

    n0 = n_static + NW

    def kv_body(w, c):
        n = n_static + w

        @pl.when(w < NW - 2)
        def _():
            win_kv(w + 1)[0](1, slot(n + 1))

        @pl.when(w == NW - 2)
        def _():
            win_kv(NW - 1)[0](1, slot(n_static + NW - 1), last=True)

        @pl.when(w == NW - 1)
        def _():
            wo_windows[0][0](1, slot(n0))

        @pl.when(w == 0)
        def _():
            win_kv(0)[2](slot(n_static), first=True)

        @pl.when(jnp.logical_and(w > 0, w < NW - 1))
        def _():
            win_kv(w)[2](slot(n))

        @pl.when(w == NW - 1)
        def _():
            win_kv(NW - 1)[2](slot(n_static + NW - 1), last=True)

        stage_head(2 * w)

        @pl.when(w < NW - 2)
        def _():
            win_kv(w + 2)[0](0, slot(n + 2))

        @pl.when(w == NW - 2)
        def _():
            wo_windows[0][0](0, slot(n0))

        @pl.when(w == NW - 1)
        def _():
            wo_windows[1][0](0, slot(n0 + 1))

        stage_head(2 * w + 1)

        @pl.when(w < DC // 128)
        def _():
            stage_ctx(w)
        return c
    jax.lax.fori_loop(0, NW, kv_body, 0)

    NJ = M // 128
    acc = [[jnp.zeros((8, 128), F32) for _ in range(NJ)] for _ in range(2)]

    def wo_head(buf, p):
        return buf[pl.ds(p * WO_TILES, WO_TILES)].reshape(16, NJ, 8, 128)

    def project(k, lo=0, hi=None):
        _, _, heads_a, heads_b = wo_windows[k]
        for n in range(lo, max(len(heads_a), len(heads_b)) if hi is None else hi):
            if n < len(heads_a):
                h, p = heads_a[n]
                ctx_h = jnp.broadcast_to(ctx_scr[h:h + 1, :], (8, D)).astype(BF16)
                w = wo_head(woa, p)
                for j in range(NJ):
                    acc[0][j] = acc[0][j] + jnp.dot(ctx_h, w[:, j].reshape(128, 128),
                                                    preferred_element_type=F32)
            if n < len(heads_b):
                h, p = heads_b[n]
                o_h = o_scr[h].astype(BF16)
                w = wo_head(wob, p)
                for j in range(NJ):
                    acc[1][j] = acc[1][j] + jnp.dot(o_h, w[:, j].reshape(128, 128),
                                                    preferred_element_type=F32)

    def wo_issue(k):
        wo_windows[k][0](0, slot(n0 + k))

    def wo_wait(k):
        wo_windows[k][1](slot(n0 + k))

    wo_issue(2)
    wo_wait(0)
    project(0, 0, 8)
    wo_issue(3)
    project(0, 8, 16)
    wo_wait(1)
    wo_issue(4)
    project(1)
    wo_wait(2)
    wo_issue(5)
    project(2)
    for k in (3, 4, 5):
        wo_wait(k)
        project(k)
    acc_a, acc_b = (jnp.concatenate(a, axis=1) for a in acc)

    out = g * acc_a[0:1, :] + (1.0 - g) * acc_b[0:1, :]
    o_ref[0] = out.astype(o_ref.dtype)


def _tiles(w):
    r, c = w.shape
    return w.reshape(r // 8, 8, c // 128, 128).transpose(0, 2, 1, 3).reshape(r // 8 * (c // 128), 8, 128)


@jax.jit
def pallas_gated_mix__compressed_kv_cla__gqa_block_cached__decode_kernel(
    A_x: jax.Array,
    A_c_kv: jax.Array,
    A_w_q: jax.Array,
    A_w_uk: jax.Array,
    A_w_uv: jax.Array,
    A_w_o: jax.Array,
    B_x: jax.Array,
    B_k_cache: jax.Array,
    B_v_cache: jax.Array,
    B_wq: jax.Array,
    B_wo: jax.Array,
    gate_w: jax.Array,
):
    del B_x
    any_spec = pl.BlockSpec(memory_space=pl.ANY)
    return pl.pallas_call(
        _kernel,
        out_shape=jax.ShapeDtypeStruct((1, 1, M), A_x.dtype),
        in_specs=[any_spec] * 11,
        out_specs=pl.BlockSpec(memory_space=pltpu.VMEM),
        scratch_shapes=[
            pltpu.VMEM((1, 1, M), BF16),
            pltpu.VMEM((M,), BF16),
            pltpu.VMEM((SK, DC), BF16),
            pltpu.VMEM((M, H, D), BF16),
            pltpu.VMEM((DC, H, D), BF16),
            pltpu.VMEM((DC, H, D), BF16),
            pltpu.VMEM((H * WO_TILES, 8, 128), BF16),
            pltpu.VMEM((H * SK, D), BF16),
            pltpu.VMEM((H * SK, D), BF16),
            pltpu.VMEM((WQ_TILES, 8, 128), BF16),
            pltpu.VMEM((H * WO_TILES, 8, 128), BF16),
            pltpu.VMEM((M, 128), F32),
            pltpu.VMEM((H, 8, D), F32),
            pltpu.VMEM((H, D), F32),
            pltpu.VMEM((H, DC), F32),
            pltpu.VMEM((H, SK), F32),
            pltpu.VMEM((DC // 128, H, 128), F32),
            pltpu.VMEM((H, D), F32),
            pltpu.VMEM((H, 8, D), F32),
            pltpu.SemaphoreType.DMA((RING,)),
            pltpu.SemaphoreType.DMA((RING,)),
        ],
        compiler_params=pltpu.CompilerParams(vmem_limit_bytes=112 * 1024 * 1024),
    )(A_x, A_c_kv, A_w_q, A_w_uk, A_w_uv, _tiles(A_w_o.reshape(H * D, M)),
      B_k_cache.reshape(H * SK, D), B_v_cache.reshape(H * SK, D),
      _tiles(B_wq), _tiles(B_wo), gate_w)
```
